```python
import jax
import jax.numpy as jnp

def _softmax(x, axis=-1):
    return jax.nn.softmax(x, axis=axis)

def _gelu(x):
    return jax.nn.gelu(x, approximate=True)

def _silu(x):
    return jax.nn.silu(x)

def _sigmoid(x):
    return jax.nn.sigmoid(x)

def _layernorm(x, axis=-1, eps=1e-05):
    m = jnp.mean(x, axis=axis, keepdims=True)
    v = jnp.var(x, axis=axis, keepdims=True)
    return (x - m) / jnp.sqrt(v + eps)

def _scatter_add(tgt, idx, src, axis=0):
    return tgt.at[idx].add(src)

def _segment_sum(src, seg, n):
    return jax.ops.segment_sum(src, seg, n)

class _Rng:

    def __init__(self, key):
        self._k = key

    def _next(self):
        self._k, sub = jax.random.split(self._k)
        return sub

    def normal(self, shape):
        return jax.random.normal(self._next(), shape, dtype=jnp.bfloat16)

    def randint(self, lo, hi, shape):
        return jax.random.randint(self._next(), shape, lo, hi, dtype=jnp.int32)

    def uniform(self, shape, lo=0.0, hi=1.0):
        return jax.random.uniform(self._next(), shape, jnp.bfloat16, lo, hi)

    def permutation(self, n):
        return jax.random.permutation(self._next(), n)
kernel_name = 'adaLN_cond__compressed_kv_cla__mixer_s_mlp__prompt'

def setup_inputs():
    _rng = _Rng(jax.random.key(int.from_bytes(__import__("os").urandom(4), "little")))
    _w = lambda a: (lambda t: t.astype(jnp.bfloat16) if jnp.issubdtype(t.dtype, jnp.floating) else t)(jnp.asarray(a))

    def _A_setup():
        B, H, Sq, Sk, D, M = (1, 32, 2048, 2048, 128, 640)
        Dc = 4 * D
        return {'x': _w((lambda *s: _rng.normal(s) * 0.05)(B, Sq, M)), 'c_kv': _w((lambda *s: _rng.normal(s) * 0.05)(B, Sk, Dc)), 'w_q': _w((lambda *s: _rng.normal(s) * 0.05)(M, H, D) * M ** (-0.5)), 'w_uk': _w((lambda *s: _rng.normal(s) * 0.05)(Dc, H, D) * Dc ** (-0.5)), 'w_uv': _w((lambda *s: _rng.normal(s) * 0.05)(Dc, H, D) * Dc ** (-0.5)), 'w_o': _w((lambda *s: _rng.normal(s) * 0.05)(H, D, M) * (H * D) ** (-0.5))}
    _A_in = _A_setup()

    def _B_setup():
        B, S, D, F = (1, 2048, 640, 1728)
        return {'x': _w((lambda *s: _rng.normal(s) * 0.05)(B, S, D)), 'w1': _w((lambda *s: _rng.normal(s) * 0.05)(D, D) * D ** (-0.5)), 'w2': _w((lambda *s: _rng.normal(s) * 0.05)(D, D) * D ** (-0.5)), 'w3': _w((lambda *s: _rng.normal(s) * 0.05)(D, F) * D ** (-0.5)), 'w4': _w((lambda *s: _rng.normal(s) * 0.05)(F, D) * F ** (-0.5))}
    _B_in = _B_setup()
    return {'A_x': _A_in['x'], 'A_c_kv': _A_in['c_kv'], 'A_w_q': _A_in['w_q'], 'A_w_uk': _A_in['w_uk'], 'A_w_uv': _A_in['w_uv'], 'A_w_o': _A_in['w_o'], 'B_x': _B_in['x'], 'B_w1': _B_in['w1'], 'B_w2': _B_in['w2'], 'B_w3': _B_in['w3'], 'B_w4': _B_in['w4'], 'c': _w((lambda *s: _rng.normal(s) * 0.05)(1, 640)), 'w_mod': _w((lambda *s: _rng.normal(s) * 0.05)(640, 6 * 640) * 640 ** (-0.5))}

def reference(A_x, A_c_kv, A_w_q, A_w_uk, A_w_uv, A_w_o, B_x, B_w1, B_w2, B_w3, B_w4, c, w_mod):

    def _A_ref(x, c_kv, w_q, w_uk, w_uv, w_o):
        B, Sq, M = (x.shape[0], x.shape[1], x.shape[2])
        Sk = c_kv.shape[1]
        H, D = (w_q.shape[1], w_q.shape[2])
        q = jnp.einsum('bqm,mhd->bhqd', x, w_q)
        k = jnp.einsum('bkc,chd->bhkd', c_kv, w_uk)
        v = jnp.einsum('bkc,chd->bhkd', c_kv, w_uv)
        scores = jnp.einsum('bhqd,bhkd->bhqk', q, k) * D ** (-0.5)
        off = Sk - Sq
        qi = jnp.arange(Sq)[:, None]
        kj = jnp.arange(Sk)[None, :]
        cmask = kj <= qi + off
        scores = jnp.where(cmask[None, None], scores, -1000000000.0)
        p = _softmax(scores, axis=-1)
        ctx = jnp.einsum('bhqk,bhkd->bhqd', p, v)
        return jnp.einsum('bhqd,hdm->bqm', ctx, w_o)

    def _B_ref(x, w1, w2, w3, w4):
        B, S, D = x.shape
        h = _gelu(_layernorm(x, axis=-1) @ w1)
        c = D // 4
        g0 = jnp.pad(h[:, :, 0 * c:1 * c], ((0, 0), (1, 0), (0, 0)))[:, :S, :]
        g1 = jnp.pad(h[:, :, 1 * c:2 * c], ((0, 0), (0, 1), (0, 0)))[:, 1:, :]
        g2 = jnp.pad(h[:, :, 2 * c:3 * c], ((0, 0), (2, 0), (0, 0)))[:, :S, :]
        g3 = jnp.pad(h[:, :, 3 * c:], ((0, 0), (0, 2), (0, 0)))[:, 2:, :]
        hs = jnp.concatenate([g0, g1, g2, g3], axis=-1) @ w2
        x1 = x + hs
        h2 = _gelu(_layernorm(x1, axis=-1) @ w3) @ w4
        return x1 + h2
    x = A_x
    mod = (_silu(c) @ w_mod).reshape(c.shape[0], 6, 1, -1)
    sa, ca, ga, sb, cb, gb = (mod[:, 0].copy(), mod[:, 1].copy(), mod[:, 2].copy(), mod[:, 3].copy(), mod[:, 4].copy(), mod[:, 5].copy())
    h = _layernorm(x, axis=-1) * (1 + ca) + sa
    x = x + ga * _A_ref(h, A_c_kv, A_w_q, A_w_uk, A_w_uv, A_w_o)
    h = _layernorm(x, axis=-1) * (1 + cb) + sb
    x = x + gb * _B_ref(h, B_w1, B_w2, B_w3, B_w4)
    return x
```

```python
import jax
import jax.numpy as jnp
import jax.experimental.pallas as pl
import jax.experimental.pallas.tpu as pltpu

S = 2048
M = 640
H = 32
D = 128
DC = 512
F = 1728
NP = H // 2
LOG2E = 1.4426950408889634
F32 = jnp.float32
BF16 = jnp.bfloat16
U32 = jnp.uint32


def _ln(x, eps=1e-5):
    m = jnp.mean(x, axis=-1, keepdims=True)
    xc = x - m
    v = jnp.mean(xc * xc, axis=-1, keepdims=True)
    return xc * jax.lax.rsqrt(v + eps)


def _gelu(x):
    return 0.5 * x * (1.0 + jnp.tanh(0.7978845608028654 * (x + 0.044715 * (x * x * x))))


def _dot(a, b):
    return jnp.dot(a, b, preferred_element_type=F32)


def _dot_nt(a, b):
    return jax.lax.dot_general(a, b, (((1,), (1,)), ((), ())), preferred_element_type=F32)


def _pk(x):
    return pltpu.bitcast(x.astype(BF16), U32)


def _upk(u):
    return pltpu.bitcast(u, BF16)


def make_kernel(R=128, KC=512, NB=2, PIN2=3, PROJ_RB=1024, EP_RB=512, NPR=NP, EPI=1):
    NC = S // R
    qscale = (D ** -0.5) * LOG2E

    def kernel(x_hbm, ckv_hbm, wq_hbm, wuk_hbm, wuv_hbm, wo_hbm, w1_hbm, w2_hbm, w3_hbm, w4_hbm,
               c_ref, wmod_hbm, z_ref, out_hbm,
               x_s, ckv_s, wo_s, w1_s, w2_s, w3_s, w4_s, wm1_s, wm2_s,
               rq_s, rk_s, rv_s, wqp_s, wkp_s, wvp_s,
               mod_s, h_s, q_s, k_s, v_s, ctx_s, x1_s, hb_s, g_s, o_s, cap_s,
               sems, rsems, osems, *bufs):
        sbufs, mbufs = bufs[0:NB], bufs[NB:2 * NB]

        wq_u = wq_hbm.bitcast(U32)
        wuk_u = wuk_hbm.bitcast(U32)
        wuv_u = wuv_hbm.bitcast(U32)

        def raw_copies(p, slot):
            return [pltpu.make_async_copy(wuk_u.at[:, p, :], rk_s.at[slot], rsems.at[slot, 0]),
                    pltpu.make_async_copy(wuv_u.at[:, p, :], rv_s.at[slot], rsems.at[slot, 1]),
                    pltpu.make_async_copy(wq_u.at[:, p, :], rq_s.at[slot], rsems.at[slot, 2])]

        cp_ckv = pltpu.make_async_copy(ckv_hbm, ckv_s, sems.at[0])
        cp_wm1 = pltpu.make_async_copy(wmod_hbm.at[:, 0:2 * M], wm1_s, sems.at[1])
        cp_x = pltpu.make_async_copy(x_hbm, x_s, sems.at[2])
        late = [pltpu.make_async_copy(wmod_hbm.at[:, 2 * M:6 * M], wm2_s, sems.at[3]),
                pltpu.make_async_copy(wo_hbm, wo_s, sems.at[4]),
                pltpu.make_async_copy(w1_hbm, w1_s, sems.at[5]),
                pltpu.make_async_copy(w2_hbm, w2_s, sems.at[6]),
                pltpu.make_async_copy(w3_hbm, w3_s, sems.at[7]),
                pltpu.make_async_copy(w4_hbm, w4_s, sems.at[8])]

        cp_ckv.start()
        for cp in raw_copies(0, 0):
            cp.start()
        cp_wm1.start()
        cp_x.start()
        for cp in raw_copies(1, 1):
            cp.start()

        def unpack(slot):
            for (src, dst, rows) in ((rk_s, wkp_s, DC), (rv_s, wvp_s, DC), (rq_s, wqp_s, M)):
                CH = 128
                for c0 in range(0, rows, CH):
                    a = src[slot, c0:c0 + CH, :]
                    lo = pltpu.bitcast(a << 16, F32)
                    hi = pltpu.bitcast(a & jnp.uint32(0xFFFF0000), F32)
                    dst[c0 // 2:(c0 + CH) // 2, 0:128] = _pk(lo)
                    dst[c0 // 2:(c0 + CH) // 2, 128:256] = _pk(hi)

        def proj_kv(r0, n):
            ck = ckv_s[pl.ds(r0, n), :]
            k = _dot(ck, _upk(wkp_s[...]))
            v = _dot(ck, _upk(wvp_s[...]))
            h0 = r0 // 2
            for hh in range(2):
                k_s[hh, pl.ds(h0, n // 2), :] = _pk(k[:, hh * D:(hh + 1) * D])
                v_s[hh, pl.ds(h0, n // 2), :] = _pk(v[:, hh * D:(hh + 1) * D])

        def proj_q(r0, n):
            h0 = r0 // 2
            q = _dot(_upk(h_s[pl.ds(h0, n // 2), :]), _upk(wqp_s[...])) * qscale
            for hh in range(2):
                q_s[hh, pl.ds(h0, n // 2), :] = _pk(q[:, hh * D:(hh + 1) * D])

        ri = jax.lax.broadcasted_iota(jnp.int32, (R, 128), 0)
        ci = jax.lax.broadcasted_iota(jnp.int32, (R, 128), 1)
        cap_s[...] = jnp.where(ci <= ri, jnp.finfo(F32).max, -1e9).astype(F32)

        cvec = c_ref[...].astype(F32)
        sc16 = jnp.broadcast_to((cvec * jax.nn.sigmoid(cvec)).astype(BF16), (16, M))

        cp_ckv.wait()
        for cp in raw_copies(0, 0):
            cp.wait()
        unpack(0)
        cp_wm1.wait()
        mod1 = _dot(sc16, wm1_s[...])[0:8].astype(BF16).astype(F32)
        sa = mod1[0:1, 0:M]
        ca1 = 1.0 + mod1[0:1, M:2 * M]
        cp_x.wait()
        for cp in late:
            cp.start()
        LNB = 256
        for i in range(S // PROJ_RB):
            proj_kv(i * PROJ_RB, PROJ_RB)
            for r0 in range(i * PROJ_RB, (i + 1) * PROJ_RB, LNB):
                xb = x_s[r0:r0 + LNB, :].astype(F32)
                h_s[r0 // 2:(r0 + LNB) // 2, :] = _pk(_ln(xb) * ca1 + sa)
        for i in range(S // PROJ_RB):
            proj_q(i * PROJ_RB, PROJ_RB)

        zst = pl.multiple_of(z_ref[0], 8)
        zld = pl.multiple_of(z_ref[1], 8)
        dfalse_h = jax.lax.broadcasted_iota(jnp.int32, (R // 2, 128), 1) < z_ref[0]
        items = [(hh, r) for hh in range(2) for r in range(NC - 1, -1, -1)]
        n_items = len(items)

        def attention(p):
            pins = {}

            def stage_a(t):
                hh, r = items[t]
                W = R * (r + 1)
                sb = sbufs[t % NB]
                qu = q_s[hh, r * R // 2:(r + 1) * R // 2, :]
                if PIN2 and (t - PIN2) in pins:
                    qu = jnp.where(dfalse_h, pins[t - PIN2], qu)
                qv = _upk(qu)
                mx = None
                for c0 in range(0, W, KC):
                    w = min(KC, W - c0)
                    sc_ = _dot_nt(qv, _upk(k_s[hh, c0 // 2:(c0 + w) // 2, :]))
                    for c1 in range(0, w, 128):
                        tile = sc_[:, c1:c1 + 128]
                        kk = c0 + c1
                        if kk == r * R:
                            tile = jnp.minimum(tile, cap_s[...])
                        sb[pl.ds(zst, R), kk:kk + 128] = tile
                        mx = tile if mx is None else jnp.maximum(mx, tile)
                mrow = jnp.max(mx, axis=-1, keepdims=True)
                mbufs[t % NB][pl.ds(zst, R), :] = jnp.broadcast_to(mrow, (R, 128))

            def stage_f(t):
                hh, r = items[t]
                W = R * (r + 1)
                sb = sbufs[t % NB]
                mn = mbufs[t % NB][pl.ds(zld, R), :]
                psum = None
                pv = None
                for c0 in range(0, W, KC):
                    w = min(KC, W - c0)
                    prs = []
                    for c1 in range(0, w, 128):
                        kk = c0 + c1
                        pr = jnp.exp2(sb[pl.ds(zld, R), kk:kk + 128] - mn)
                        psum = pr if psum is None else psum + pr
                        prs.append(pr)
                    pm = (prs[0] if len(prs) == 1 else jnp.concatenate(prs, axis=1)).astype(BF16)
                    d = _dot(pm, _upk(v_s[hh, c0 // 2:(c0 + w) // 2, :]))
                    pv = d if pv is None else pv + d
                lt = jnp.sum(psum, axis=-1, keepdims=True)
                o = _pk(pv * (1.0 / lt))
                pins[t] = o
                ctx_s[p, r * R // 2:(r + 1) * R // 2, hh * D:(hh + 1) * D] = o

            for t in range(n_items + 1):
                if t < n_items:
                    stage_a(t)
                if t >= 1:
                    stage_f(t - 1)

        def pair_body(p, _):
            @pl.when(p + 2 < NP)
            def _start():
                for cp in raw_copies(p + 2, p % 2):
                    cp.start()
            nslot = (p + 1) % 2
            for cp in raw_copies(p + 1, nslot):
                cp.wait()
            unpack(nslot)
            attention(p)
            for i in range(S // PROJ_RB):
                proj_kv(i * PROJ_RB, PROJ_RB)
                proj_q(i * PROJ_RB, PROJ_RB)
            return _

        jax.lax.fori_loop(0, NPR - 1, pair_body, None)
        attention(NP - 1)

        for cp in late:
            cp.wait()
        mod2 = _dot(sc16, wm2_s[...])[0:8].astype(BF16).astype(F32)
        mod_s[...] = mod2

        g_s[0:8, :] = jnp.zeros((8, M), F32)
        g_s[8 + S:16 + S, :] = jnp.zeros((8, M), F32)

        def ep1_body(r, _):
            r0 = pl.multiple_of(r * EP_RB, EP_RB)
            rs = pl.ds(r0, EP_RB)
            rs2 = pl.ds(pl.multiple_of(r * (EP_RB // 2), EP_RB // 2), EP_RB // 2)
            acc = None
            for pp in range(NP):
                d = _dot(_upk(ctx_s[pp, rs2, :]), wo_s[pp])
                acc = d if acc is None else acc + d
            ga = mod_s[0:1, 0:M]
            sb_ = mod_s[0:1, M:2 * M]
            cb = mod_s[0:1, 2 * M:3 * M]
            x1 = x_s[rs, :].astype(F32) + ga * acc
            x1_s[rs, :] = x1
            hb = _ln(x1) * (1.0 + cb) + sb_
            hb_s[rs, :] = hb
            g = _gelu(_dot(_ln(hb).astype(BF16), w1_s[...]))
            g_s[pl.ds(r0 + 8, EP_RB), :] = g
            return _

        def ep2_body(r, _):
            r0 = pl.multiple_of(r * EP_RB, EP_RB)
            rs = pl.ds(r0, EP_RB)

            @pl.when(r >= 2)
            def _w():
                pltpu.make_async_copy(o_s.at[r % 2], out_hbm.at[pl.ds(pl.multiple_of((r - 2) * EP_RB, EP_RB), EP_RB), :],
                                      osems.at[r % 2]).wait()
            lane = jax.lax.broadcasted_iota(jnp.int32, (EP_RB, 128), 1)
            wins = {c0: g_s[pl.ds(r0, EP_RB + 16), c0:c0 + 128] for c0 in range(0, M, 128)}
            gm1 = lambda c0: wins[c0][7:7 + EP_RB]
            gp1 = lambda c0: wins[c0][9:9 + EP_RB]
            gm2 = lambda c0: wins[c0][6:6 + EP_RB]
            gp2 = lambda c0: wins[c0][10:10 + EP_RB]
            t0 = gm1(0)
            t1 = jnp.where(lane < 32, gm1(128), gp1(128))
            t2 = jnp.where(lane < 64, gp1(256), gm2(256))
            t3 = jnp.where(lane < 96, gm2(384), gp2(384))
            t4 = gp2(512)
            gs = jnp.concatenate([t0, t1, t2, t3, t4], axis=1).astype(BF16)
            xb = hb_s[rs, :] + _dot(gs, w2_s[...])
            u = _gelu(_dot_nt(_ln(xb).astype(BF16), w3_s[...])).astype(BF16)
            h2 = _dot(u, w4_s[...])
            gb = mod_s[0:1, 3 * M:4 * M]
            o = x1_s[rs, :] + gb * (xb + h2)
            o_s[r % 2] = o.astype(BF16)
            pltpu.make_async_copy(o_s.at[r % 2], out_hbm.at[rs, :], osems.at[r % 2]).start()
            return _

        NE = S // EP_RB
        if EPI:
            jax.lax.fori_loop(0, NE, ep1_body, None)
            jax.lax.fori_loop(0, NE, ep2_body, None)
            for r in (NE - 2, NE - 1):
                pltpu.make_async_copy(o_s.at[r % 2], out_hbm.at[pl.ds(r * EP_RB, EP_RB), :], osems.at[r % 2]).wait()
        else:
            o_s[0] = _upk(ctx_s[0, 0:EP_RB // 2, 0:128]).astype(BF16)[:, 0:1] + jnp.zeros((EP_RB, M), BF16)
            cpo = pltpu.make_async_copy(o_s.at[0], out_hbm.at[pl.ds(0, EP_RB), :], osems.at[0])
            cpo.start()
            cpo.wait()

    return kernel


def run(A_x, A_c_kv, A_w_q, A_w_uk, A_w_uv, A_w_o, B_x, B_w1, B_w2, B_w3, B_w4, c, w_mod, **kw):
    EP_RB = kw.get("EP_RB", 512)
    R = kw.get("R", 128)
    NB = kw.get("NB", 2)
    flags = {}
    if kw.pop("LP", 1):
        flags["XLA_TPU_FORCE_LP_LLO_SCHEDULER"] = True
    kernel = make_kernel(**kw)
    hbm = pl.BlockSpec(memory_space=pltpu.HBM)
    out = pl.pallas_call(
        kernel,
        out_shape=jax.ShapeDtypeStruct((S, M), BF16),
        in_specs=[hbm] * 10 + [pl.BlockSpec(memory_space=pltpu.VMEM), hbm, pl.BlockSpec(memory_space=pltpu.SMEM)],
        out_specs=hbm,
        scratch_shapes=[
            pltpu.VMEM((S, M), BF16), pltpu.VMEM((S, DC), BF16),
            pltpu.VMEM((NP, 2 * D, M), BF16),
            pltpu.VMEM((M, M), BF16), pltpu.VMEM((M, M), BF16), pltpu.VMEM((F, M), BF16), pltpu.VMEM((F, M), BF16),
            pltpu.VMEM((M, 2 * M), BF16), pltpu.VMEM((M, 4 * M), BF16),
            pltpu.VMEM((2, M, D), U32), pltpu.VMEM((2, DC, D), U32), pltpu.VMEM((2, DC, D), U32),
            pltpu.VMEM((M // 2, 2 * D), U32), pltpu.VMEM((DC // 2, 2 * D), U32), pltpu.VMEM((DC // 2, 2 * D), U32),
            pltpu.VMEM((8, 4 * M), F32),
            pltpu.VMEM((S // 2, M), U32),
            pltpu.VMEM((2, S // 2, D), U32), pltpu.VMEM((2, S // 2, D), U32), pltpu.VMEM((2, S // 2, D), U32),
            pltpu.VMEM((NP, S // 2, 2 * D), U32),
            pltpu.VMEM((S, M), F32),
            pltpu.VMEM((S, M), F32),
            pltpu.VMEM((S + 16, M), F32),
            pltpu.VMEM((2, EP_RB, M), BF16),
            pltpu.VMEM((R, 128), F32),
            pltpu.SemaphoreType.DMA((9,)),
            pltpu.SemaphoreType.DMA((2, 3)),
            pltpu.SemaphoreType.DMA((2,)),
        ] + [pltpu.VMEM((R, S), F32)] * NB + [pltpu.VMEM((R, 128), F32)] * NB,
        compiler_params=pltpu.CompilerParams(vmem_limit_bytes=120 * 1024 * 1024, flags=flags),
    )(A_x.reshape(S, M), A_c_kv.reshape(S, DC), A_w_q, A_w_uk, A_w_uv, A_w_o.reshape(NP, 2 * D, M),
      B_w1, B_w2, B_w3.T, B_w4, c, w_mod, jnp.zeros((2,), jnp.int32))
    return out.reshape(1, S, M)


@jax.jit
def pallas_adaLN_cond__compressed_kv_cla__mixer_s_mlp__prompt_kernel(
    A_x: jax.Array,
    A_c_kv: jax.Array,
    A_w_q: jax.Array,
    A_w_uk: jax.Array,
    A_w_uv: jax.Array,
    A_w_o: jax.Array,
    B_x: jax.Array,
    B_w1: jax.Array,
    B_w2: jax.Array,
    B_w3: jax.Array,
    B_w4: jax.Array,
    c: jax.Array,
    w_mod: jax.Array,
):
    return run(A_x, A_c_kv, A_w_q, A_w_uk, A_w_uv, A_w_o, B_x, B_w1, B_w2, B_w3, B_w4, c, w_mod)
```

```python
import jax
import jax.numpy as jnp
import jax.experimental.pallas as pl
import jax.experimental.pallas.tpu as pltpu

S = 2048
M = 640
H = 32
D = 128
DC = 512
F = 1728
NP = H // 2
LOG2E = 1.4426950408889634
F32 = jnp.float32
BF16 = jnp.bfloat16
U32 = jnp.uint32


def _ln(x, eps=1e-5):
    m = jnp.mean(x, axis=-1, keepdims=True)
    xc = x - m
    v = jnp.mean(xc * xc, axis=-1, keepdims=True)
    return xc * jax.lax.rsqrt(v + eps)


def _gelu(x):
    return 0.5 * x * (1.0 + jnp.tanh(0.7978845608028654 * (x + 0.044715 * (x * x * x))))


def _dot(a, b):
    return jnp.dot(a, b, preferred_element_type=F32)


def _dot_nt(a, b):
    return jax.lax.dot_general(a, b, (((1,), (1,)), ((), ())), preferred_element_type=F32)


def _pk(x):
    return pltpu.bitcast(x.astype(BF16), U32)


def _upk(u):
    return pltpu.bitcast(u, BF16)


def make_kernel(R=128, KC=512, NB=2, PIN2=3, PROJ_RB=1024, EP_RB=512, NPR=NP, EPI=1, GRP=4, UNP=3, HOIST=1, PRO=1, EP1_RB=512, NODMA=0):
    NC = S // R
    qscale = (D ** -0.5) * LOG2E

    def kernel(x_hbm, ckv_hbm, wq_hbm, wuk_hbm, wuv_hbm, wo_hbm, w1_hbm, w2_hbm, w3_hbm, w4_hbm,
               c_ref, wmod_hbm, z_ref, out_hbm,
               x_s, ckv_s, wo_s, w1_s, w2_s, w3_s, w4_s, wm1_s, wm2_s,
               rq_s, rk_s, rv_s, wqp_s, wkp_s, wvp_s,
               mod_s, h_s, q_s, k_s, v_s, ctx_s, x1_s, hb_s, g_s, o_s, cap_s,
               sems, rsems, osems, *bufs):
        sbufs, mbufs = bufs[0:NB], bufs[NB:2 * NB]

        wq_u = wq_hbm.bitcast(U32)
        wuk_u = wuk_hbm.bitcast(U32)
        wuv_u = wuv_hbm.bitcast(U32)

        def raw_copies(p, slot):
            return [pltpu.make_async_copy(wuk_u.at[:, p, :], rk_s.at[slot], rsems.at[slot, 0]),
                    pltpu.make_async_copy(wuv_u.at[:, p, :], rv_s.at[slot], rsems.at[slot, 1]),
                    pltpu.make_async_copy(wq_u.at[:, p, :], rq_s.at[slot], rsems.at[slot, 2])]

        cp_ckv = pltpu.make_async_copy(ckv_hbm, ckv_s, sems.at[0])
        cp_wm1 = pltpu.make_async_copy(wmod_hbm.at[:, 0:2 * M], wm1_s, sems.at[1])
        cp_x = pltpu.make_async_copy(x_hbm, x_s, sems.at[2])
        late = [pltpu.make_async_copy(wmod_hbm.at[:, 2 * M:6 * M], wm2_s, sems.at[3]),
                pltpu.make_async_copy(wo_hbm, wo_s, sems.at[4]),
                pltpu.make_async_copy(w1_hbm, w1_s, sems.at[5]),
                pltpu.make_async_copy(w2_hbm, w2_s, sems.at[6]),
                pltpu.make_async_copy(w3_hbm, w3_s, sems.at[7]),
                pltpu.make_async_copy(w4_hbm, w4_s, sems.at[8])]

        def unpack(slot, which=(0, 1, 2)):
            for (src, dst, rows) in [((rk_s, wkp_s, DC), (rv_s, wvp_s, DC), (rq_s, wqp_s, M))[w_] for w_ in which]:
                CH = 128
                for c0 in range(0, rows, CH):
                    a = src[slot, c0:c0 + CH, :]
                    lo = pltpu.bitcast(a << 16, F32)
                    hi = pltpu.bitcast(a & jnp.uint32(0xFFFF0000), F32)
                    dst[c0 // 2:(c0 + CH) // 2, 0:128] = _pk(lo)
                    dst[c0 // 2:(c0 + CH) // 2, 128:256] = _pk(hi)

        def proj_kv(r0, n):
            ck = ckv_s[pl.ds(r0, n), :]
            k = _dot(ck, _upk(wkp_s[...]))
            v = _dot(ck, _upk(wvp_s[...]))
            h0 = r0 // 2
            for hh in range(2):
                k_s[hh, pl.ds(h0, n // 2), :] = _pk(k[:, hh * D:(hh + 1) * D])
                v_s[hh, pl.ds(h0, n // 2), :] = _pk(v[:, hh * D:(hh + 1) * D])

        def proj_q(r0, n):
            h0 = r0 // 2
            q = _dot(_upk(h_s[pl.ds(h0, n // 2), :]), _upk(wqp_s[...])) * qscale
            for hh in range(2):
                q_s[hh, pl.ds(h0, n // 2), :] = _pk(q[:, hh * D:(hh + 1) * D])

        ri = jax.lax.broadcasted_iota(jnp.int32, (R, 128), 0)
        ci = jax.lax.broadcasted_iota(jnp.int32, (R, 128), 1)
        cap_s[...] = jnp.where(ci <= ri, jnp.finfo(F32).max, -1e9).astype(F32)

        cvec = c_ref[...].astype(F32)
        sc16 = jnp.broadcast_to((cvec * jax.nn.sigmoid(cvec)).astype(BF16), (16, M))

        def ln_rows(r0, n, ca1, sa):
            for a0 in range(r0, r0 + n, 256):
                xb = x_s[a0:a0 + 256, :].astype(F32)
                h_s[a0 // 2:(a0 + 256) // 2, :] = _pk(_ln(xb) * ca1 + sa)

        def mod1():
            m1 = _dot(sc16, wm1_s[...])[0:8].astype(BF16).astype(F32)
            return 1.0 + m1[0:1, M:2 * M], m1[0:1, 0:M]

        HS = S // 2
        if PRO == 0:
            cp_ckv.start()
            for cp in raw_copies(0, 0):
                cp.start()
            cp_wm1.start()
            cp_x.start()
            if NPR > 1 and not NODMA:
                for cp in raw_copies(1, 1):
                    cp.start()
            cp_ckv.wait()
            for cp in raw_copies(0, 0):
                cp.wait()
            unpack(0)
            cp_wm1.wait()
            ca1, sa = mod1()
            cp_x.wait()
            for cp in late:
                cp.start()
            for i in range(2):
                proj_kv(i * HS, HS)
                ln_rows(i * HS, HS, ca1, sa)
            for i in range(2):
                proj_q(i * HS, HS)
        else:
            raw0 = raw_copies(0, 0)
            ckv_a = pltpu.make_async_copy(ckv_hbm.at[0:HS, :], ckv_s.at[0:HS, :], sems.at[0])
            ckv_b = pltpu.make_async_copy(ckv_hbm.at[HS:S, :], ckv_s.at[HS:S, :], sems.at[9])
            raw0[0].start()
            raw0[1].start()
            ckv_a.start()
            ckv_b.start()
            if PRO == 1:
                raw0[0].wait()
                raw0[1].wait()
                ckv_a.wait()
            cp_x.start()
            cp_wm1.start()
            raw0[2].start()
            if PRO == 2:
                raw0[0].wait()
                raw0[1].wait()
                ckv_a.wait()
            unpack(0, (0, 1))
            proj_kv(0, HS)
            ckv_b.wait()
            proj_kv(HS, HS)
            cp_wm1.wait()
            cp_x.wait()
            raw0[2].wait()
            if NPR > 1 and not NODMA:
                for cp in raw_copies(1, 1):
                    cp.start()
            if NPR < 3:
                for cp in late:
                    cp.start()
            unpack(0, (2,))
            ca1, sa = mod1()
            for i in range(4):
                ln_rows(i * HS // 2, HS // 2, ca1, sa)
                proj_q(i * HS // 2, HS // 2)

        zst = pl.multiple_of(z_ref[0], 8)
        zld = pl.multiple_of(z_ref[1], 8)
        dfalse_h = jax.lax.broadcasted_iota(jnp.int32, (R // 2, 128), 1) < z_ref[0]
        if GRP == 0:
            seq = [[r] for r in range(NC - 1, -1, -1)]
        elif GRP == 1:
            seq = [[r] for r in range(15, 3, -1)] + [[3, 2, 1, 0]]
        elif GRP == 2:
            seq = [[r] for r in range(15, 7, -1)] + [[7, 0], [6, 1], [5, 2], [4, 3]]
        elif GRP == 3:
            seq = [[15], [14], [13], [12, 0], [11, 1], [10, 2], [9, 3], [8, 4], [7, 5], [6]]
        elif GRP == 4:
            seq = [[15], [14, 0], [13, 1], [12, 2], [11, 3], [10, 4], [9, 5], [8, 6], [7]]
        items = [(hh, rs) for hh in range(2) for rs in seq]
        n_items = len(items)
        MAXP = max(len(rs) for rs in seq)

        def attention(p, extra=None):
            pins = {}

            def stage_a(t):
                hh, rs = items[t]
                sb = sbufs[t % NB]
                off = 0
                for pi, r in enumerate(rs):
                    W = R * (r + 1)
                    qu = q_s[hh, r * R // 2:(r + 1) * R // 2, :]
                    if PIN2 and (t - PIN2) in pins and pi == 0:
                        for o_prev in pins[t - PIN2]:
                            qu = jnp.where(dfalse_h, o_prev, qu)
                    qv = _upk(qu)
                    mx = None
                    for c0 in range(0, W, KC):
                        w = min(KC, W - c0)
                        sc_ = _dot_nt(qv, _upk(k_s[hh, c0 // 2:(c0 + w) // 2, :]))
                        for c1 in range(0, w, 128):
                            tile = sc_[:, c1:c1 + 128]
                            kk = c0 + c1
                            if kk == r * R:
                                tile = jnp.minimum(tile, cap_s[...])
                            sb[pl.ds(zst, R), off + kk:off + kk + 128] = tile
                            mx = tile if mx is None else jnp.maximum(mx, tile)
                    mrow = jnp.max(mx, axis=-1, keepdims=True)
                    mbufs[t % NB][pl.ds(zst, R), pi * 128:(pi + 1) * 128] = jnp.broadcast_to(mrow, (R, 128))
                    off += W

            def stage_f(t):
                hh, rs = items[t]
                sb = sbufs[t % NB]
                off = 0
                pins[t] = []
                for pi, r in enumerate(rs):
                    W = R * (r + 1)
                    mn = mbufs[t % NB][pl.ds(zld, R), pi * 128:(pi + 1) * 128]
                    psum = None
                    pv = None
                    for c0 in range(0, W, KC):
                        w = min(KC, W - c0)
                        prs = []
                        for c1 in range(0, w, 128):
                            kk = off + c0 + c1
                            pr = jnp.exp2(sb[pl.ds(zld, R), kk:kk + 128] - mn)
                            psum = pr if psum is None else psum + pr
                            prs.append(pr)
                        pm = (prs[0] if len(prs) == 1 else jnp.concatenate(prs, axis=1)).astype(BF16)
                        d = _dot(pm, _upk(v_s[hh, c0 // 2:(c0 + w) // 2, :]))
                        pv = d if pv is None else pv + d
                    lt = jnp.sum(psum, axis=-1, keepdims=True)
                    r0_ = pl.reciprocal(lt, approx=True)
                    rl = r0_ * (2.0 - lt * r0_)
                    o = _pk(pv * rl)
                    pins[t].append(o)
                    ctx_s[p, r * R // 2:(r + 1) * R // 2, hh * D:(hh + 1) * D] = o
                    off += W

            for t in range(n_items + 1):
                if t < n_items:
                    stage_a(t)
                if extra is not None and t in extra:
                    extra[t]()
                if t >= 1:
                    stage_f(t - 1)

        def pair_body(p, _):
            @pl.when((p + 2 < NPR) & (NODMA == 0))
            def _start():
                for cp in raw_copies(p + 2, p % 2):
                    cp.start()
            nslot = (p + 1) % 2

            @pl.when((p == 1) & (NPR >= 3))
            def _late():
                for cp in late:
                    cp.start()

            if not NODMA:
                for cp in raw_copies(p + 1, nslot):
                    cp.wait()

            def wait_unpack():
                unpack(nslot)
            pieces = []
            for i in range(S // PROJ_RB - 1, -1, -1):
                pieces.append(lambda i=i: proj_q(i * PROJ_RB, PROJ_RB))
                pieces.append(lambda i=i: proj_kv(i * PROJ_RB, PROJ_RB))
            extra = {UNP: wait_unpack}
            used = 0
            if HOIST >= 1:
                extra[n_items] = pieces[0]
                used = 1
            if HOIST >= 2:
                extra[n_items - 1] = pieces[0]
                extra[n_items] = pieces[1]
                used = 2
            attention(p, extra)
            for f in pieces[used:]:
                f()
            return _

        jax.lax.fori_loop(0, NPR - 1, pair_body, None)
        attention(NP - 1)

        for cp in late:
            cp.wait()
        mod2 = _dot(sc16, wm2_s[...])[0:8].astype(BF16).astype(F32)
        mod_s[...] = mod2

        g_s[0:8, :] = jnp.zeros((8, M), F32)
        g_s[8 + S:16 + S, :] = jnp.zeros((8, M), F32)

        HB1 = EP1_RB // 2

        def ep1_body(r, _):
            halves = []
            for hf in range(2):
                r0 = pl.multiple_of(r * EP1_RB + hf * HB1, HB1)
                rs = pl.ds(r0, HB1)
                rs2 = pl.ds(pl.multiple_of(r * (EP1_RB // 2) + hf * (HB1 // 2), HB1 // 2), HB1 // 2)
                cx = jnp.concatenate([_upk(ctx_s[pp, rs2, :]) for pp in range(NP)], axis=1)
                halves.append((r0, rs, x_s[rs, :], _dot(cx, wo_s[...])))
            ga = mod_s[0:1, 0:M]
            sb_ = mod_s[0:1, M:2 * M]
            cb = mod_s[0:1, 2 * M:3 * M]
            outs = []
            for (r0, rs, xin, acc) in halves:
                x1 = xin.astype(F32) + ga * acc
                hb = _ln(x1) * (1.0 + cb) + sb_
                pre = _dot(_ln(hb).astype(BF16), w1_s[...])
                outs.append((r0, rs, x1, hb, pre))
            for (r0, rs, x1, hb, pre) in outs:
                g = _gelu(pre)
                x1_s[rs, :] = x1
                hb_s[rs, :] = hb
                g_s[pl.ds(r0 + 8, HB1), :] = g
            return _

        def ep2_body(r, _):
            r0 = pl.multiple_of(r * EP_RB, EP_RB)
            rs = pl.ds(r0, EP_RB)

            @pl.when(r >= 2)
            def _w():
                pltpu.make_async_copy(o_s.at[r % 2], out_hbm.at[pl.ds(pl.multiple_of((r - 2) * EP_RB, EP_RB), EP_RB), :],
                                      osems.at[r % 2]).wait()
            lane = jax.lax.broadcasted_iota(jnp.int32, (EP_RB, 128), 1)
            wins = {c0: g_s[pl.ds(r0, EP_RB + 16), c0:c0 + 128] for c0 in range(0, M, 128)}
            gm1 = lambda c0: wins[c0][7:7 + EP_RB]
            gp1 = lambda c0: wins[c0][9:9 + EP_RB]
            gm2 = lambda c0: wins[c0][6:6 + EP_RB]
            gp2 = lambda c0: wins[c0][10:10 + EP_RB]
            t0 = gm1(0)
            t1 = jnp.where(lane < 32, gm1(128), gp1(128))
            t2 = jnp.where(lane < 64, gp1(256), gm2(256))
            t3 = jnp.where(lane < 96, gm2(384), gp2(384))
            t4 = gp2(512)
            gs = jnp.concatenate([t0, t1, t2, t3, t4], axis=1).astype(BF16)
            xb = hb_s[rs, :] + _dot(gs, w2_s[...])
            u = _gelu(_dot_nt(_ln(xb).astype(BF16), w3_s[...])).astype(BF16)
            h2 = _dot(u, w4_s[...])
            gb = mod_s[0:1, 3 * M:4 * M]
            o = x1_s[rs, :] + gb * (xb + h2)
            o_s[r % 2] = o.astype(BF16)
            pltpu.make_async_copy(o_s.at[r % 2], out_hbm.at[rs, :], osems.at[r % 2]).start()
            return _

        NE = S // EP_RB
        if EPI in (1, 2):
            jax.lax.fori_loop(0, S // EP1_RB, ep1_body, None)
        if EPI in (1, 3):
            jax.lax.fori_loop(0, NE, ep2_body, None)
            for r in (NE - 2, NE - 1):
                pltpu.make_async_copy(o_s.at[r % 2], out_hbm.at[pl.ds(r * EP_RB, EP_RB), :], osems.at[r % 2]).wait()
        if EPI in (0, 2):
            o_s[0] = _upk(ctx_s[0, 0:EP_RB // 2, 0:128]).astype(BF16)[:, 0:1] + jnp.zeros((EP_RB, M), BF16)
            cpo = pltpu.make_async_copy(o_s.at[0], out_hbm.at[pl.ds(0, EP_RB), :], osems.at[0])
            cpo.start()
            cpo.wait()

    return kernel


def run(A_x, A_c_kv, A_w_q, A_w_uk, A_w_uv, A_w_o, B_x, B_w1, B_w2, B_w3, B_w4, c, w_mod, **kw):
    EP_RB = kw.get("EP_RB", 512)
    R = kw.get("R", 128)
    NB = kw.get("NB", 2)
    flags = {}
    if kw.pop("LP", 1):
        flags["XLA_TPU_FORCE_LP_LLO_SCHEDULER"] = True
    kernel = make_kernel(**kw)
    hbm = pl.BlockSpec(memory_space=pltpu.HBM)
    out = pl.pallas_call(
        kernel,
        out_shape=jax.ShapeDtypeStruct((S, M), BF16),
        in_specs=[hbm] * 10 + [pl.BlockSpec(memory_space=pltpu.VMEM), hbm, pl.BlockSpec(memory_space=pltpu.SMEM)],
        out_specs=hbm,
        scratch_shapes=[
            pltpu.VMEM((S, M), BF16), pltpu.VMEM((S, DC), BF16),
            pltpu.VMEM((H * D, M), BF16),
            pltpu.VMEM((M, M), BF16), pltpu.VMEM((M, M), BF16), pltpu.VMEM((F, M), BF16), pltpu.VMEM((F, M), BF16),
            pltpu.VMEM((M, 2 * M), BF16), pltpu.VMEM((M, 4 * M), BF16),
            pltpu.VMEM((2, M, D), U32), pltpu.VMEM((2, DC, D), U32), pltpu.VMEM((2, DC, D), U32),
            pltpu.VMEM((M // 2, 2 * D), U32), pltpu.VMEM((DC // 2, 2 * D), U32), pltpu.VMEM((DC // 2, 2 * D), U32),
            pltpu.VMEM((8, 4 * M), F32),
            pltpu.VMEM((S // 2, M), U32),
            pltpu.VMEM((2, S // 2, D), U32), pltpu.VMEM((2, S // 2, D), U32), pltpu.VMEM((2, S // 2, D), U32),
            pltpu.VMEM((NP, S // 2, 2 * D), U32),
            pltpu.VMEM((S, M), F32),
            pltpu.VMEM((S, M), F32),
            pltpu.VMEM((S + 16, M), F32),
            pltpu.VMEM((2, EP_RB, M), BF16),
            pltpu.VMEM((R, 128), F32),
            pltpu.SemaphoreType.DMA((10,)),
            pltpu.SemaphoreType.DMA((2, 3)),
            pltpu.SemaphoreType.DMA((2,)),
        ] + [pltpu.VMEM((R, S), F32)] * NB + [pltpu.VMEM((R, 512), F32)] * NB,
        compiler_params=pltpu.CompilerParams(vmem_limit_bytes=120 * 1024 * 1024, flags=flags),
    )(A_x.reshape(S, M), A_c_kv.reshape(S, DC), A_w_q, A_w_uk, A_w_uv, A_w_o.reshape(H * D, M),
      B_w1, B_w2, B_w3.T, B_w4, c, w_mod, jnp.zeros((2,), jnp.int32))
    return out.reshape(1, S, M)


@jax.jit
def pallas_adaLN_cond__compressed_kv_cla__mixer_s_mlp__prompt_kernel(
    A_x: jax.Array,
    A_c_kv: jax.Array,
    A_w_q: jax.Array,
    A_w_uk: jax.Array,
    A_w_uv: jax.Array,
    A_w_o: jax.Array,
    B_x: jax.Array,
    B_w1: jax.Array,
    B_w2: jax.Array,
    B_w3: jax.Array,
    B_w4: jax.Array,
    c: jax.Array,
    w_mod: jax.Array,
):
    return run(A_x, A_c_kv, A_w_q, A_w_uk, A_w_uv, A_w_o, B_x, B_w1, B_w2, B_w3, B_w4, c, w_mod)
```

```python
import jax
import jax.numpy as jnp
import numpy as np
import jax.experimental.pallas as pl
import jax.experimental.pallas.tpu as pltpu

S = 2048
M = 640
H = 32
D = 128
DC = 512
F = 1728
NP = H // 2
LOG2E = 1.4426950408889634
F32 = jnp.float32
BF16 = jnp.bfloat16
U32 = jnp.uint32


def _ln(x, eps=1e-5):
    m = jnp.mean(x, axis=-1, keepdims=True)
    xc = x - m
    v = jnp.mean(xc * xc, axis=-1, keepdims=True)
    return xc * jax.lax.rsqrt(v + eps)


def _gelu(x):
    return 0.5 * x * (1.0 + jnp.tanh(0.7978845608028654 * (x + 0.044715 * (x * x * x))))


def _dot(a, b):
    return jnp.dot(a, b, preferred_element_type=F32)


def _dot_nt(a, b):
    return jax.lax.dot_general(a, b, (((1,), (1,)), ((), ())), preferred_element_type=F32)


def _pk(x):
    return pltpu.bitcast(x.astype(BF16), U32)


def _upk(u):
    return pltpu.bitcast(u, BF16)


R = 128
KC = 512
NB = 2
PIN = 3
PROJ_RB = 1024
EP_RB = 512
EPH = 4
HS = S // 2


def make_kernel():
    NC = S // R
    qscale = (D ** -0.5) * LOG2E

    def kernel(x_hbm, ckv_hbm, wq_hbm, wuk_hbm, wuv_hbm, wo_hbm, w1_hbm, w2_hbm, w3_hbm, w4_hbm,
               c_ref, wmod_hbm, z_ref, out_hbm,
               x_s, ckv_s, wo_s, w1_s, w2_s, w3_s, w4_s, wm1_s, wm2_s,
               rq_s, rk_s, rv_s, wqp_s, wkp_s, wvp_s,
               mod_s, h_s, q_s, k_s, v_s, ctx_s, x1_s, hb_s, g_s, o_s, cap_s,
               sems, rsems, osems, *bufs):
        sbufs, mbufs = bufs[0:NB], bufs[NB:2 * NB]

        wq_u = wq_hbm.bitcast(U32)
        wuk_u = wuk_hbm.bitcast(U32)
        wuv_u = wuv_hbm.bitcast(U32)

        def raw_copies(p, slot):
            return [pltpu.make_async_copy(wuk_u.at[:, p, :], rk_s.at[slot], rsems.at[slot, 0]),
                    pltpu.make_async_copy(wuv_u.at[:, p, :], rv_s.at[slot], rsems.at[slot, 1]),
                    pltpu.make_async_copy(wq_u.at[:, p, :], rq_s.at[slot], rsems.at[slot, 2])]

        cp_wm1 = pltpu.make_async_copy(wmod_hbm.at[:, 0:2 * M], wm1_s, sems.at[1])
        late = [pltpu.make_async_copy(wmod_hbm.at[:, 2 * M:6 * M], wm2_s, sems.at[3]),
                pltpu.make_async_copy(wo_hbm, wo_s, sems.at[4]),
                pltpu.make_async_copy(w1_hbm, w1_s, sems.at[5]),
                pltpu.make_async_copy(w2_hbm, w2_s, sems.at[6]),
                pltpu.make_async_copy(w3_hbm, w3_s, sems.at[7]),
                pltpu.make_async_copy(w4_hbm, w4_s, sems.at[8])]

        def unpack(slot, which=(0, 1, 2)):
            for (src, dst, rows) in [((rk_s, wkp_s, DC), (rv_s, wvp_s, DC), (rq_s, wqp_s, M))[w_] for w_ in which]:
                CH = 128
                for c0 in range(0, rows, CH):
                    a = src[slot, c0:c0 + CH, :]
                    lo = pltpu.bitcast(a << 16, F32)
                    hi = pltpu.bitcast(a & jnp.uint32(0xFFFF0000), F32)
                    dst[c0 // 2:(c0 + CH) // 2, 0:128] = _pk(lo)
                    dst[c0 // 2:(c0 + CH) // 2, 128:256] = _pk(hi)

        def proj_kv(r0, n):
            ck = ckv_s[pl.ds(r0, n), :]
            k = _dot(ck, _upk(wkp_s[...]))
            v = _dot(ck, _upk(wvp_s[...]))
            h0 = r0 // 2
            for hh in range(2):
                k_s[hh, pl.ds(h0, n // 2), :] = _pk(k[:, hh * D:(hh + 1) * D])
                v_s[hh, pl.ds(h0, n // 2), :] = _pk(v[:, hh * D:(hh + 1) * D])

        def proj_q(r0, n):
            h0 = r0 // 2
            q = _dot(_upk(h_s[pl.ds(h0, n // 2), :]), _upk(wqp_s[...])) * qscale
            for hh in range(2):
                q_s[hh, pl.ds(h0, n // 2), :] = _pk(q[:, hh * D:(hh + 1) * D])

        ri = jax.lax.broadcasted_iota(jnp.int32, (R, 128), 0)
        ci = jax.lax.broadcasted_iota(jnp.int32, (R, 128), 1)
        cap_s[...] = jnp.where(ci <= ri, jnp.finfo(F32).max, -1e9).astype(F32)

        cvec = c_ref[...].astype(F32)
        sc16 = jnp.broadcast_to((cvec * jax.nn.sigmoid(cvec)).astype(BF16), (16, M))

        def ln_rows(r0, n, ca1, sa):
            for a0 in range(r0, r0 + n, 256):
                xb = x_s[a0:a0 + 256, :].astype(F32)
                h_s[a0 // 2:(a0 + 256) // 2, :] = _pk(_ln(xb) * ca1 + sa)

        def mod1():
            m1 = _dot(sc16, wm1_s[...])[0:8].astype(BF16).astype(F32)
            return 1.0 + m1[0:1, M:2 * M], m1[0:1, 0:M]

        raw0 = raw_copies(0, 0)
        ckv_a = pltpu.make_async_copy(ckv_hbm.at[0:HS, :], ckv_s.at[0:HS, :], sems.at[0])
        ckv_b = pltpu.make_async_copy(ckv_hbm.at[HS:S, :], ckv_s.at[HS:S, :], sems.at[9])
        raw0[0].start()
        raw0[1].start()
        ckv_a.start()
        ckv_b.start()
        x_a = pltpu.make_async_copy(x_hbm.at[0:HS, :], x_s.at[0:HS, :], sems.at[2])
        x_b = pltpu.make_async_copy(x_hbm.at[HS:S, :], x_s.at[HS:S, :], sems.at[10])
        raw0[0].wait()
        raw0[1].wait()
        ckv_a.wait()
        cp_wm1.start()
        x_a.start()
        raw0[2].start()
        unpack(0, (0, 1))
        proj_kv(0, HS)
        ckv_b.wait()
        x_b.start()
        for cp in raw_copies(1, 1):
            cp.start()
        proj_kv(HS, HS)
        cp_wm1.wait()
        x_a.wait()
        raw0[2].wait()
        unpack(0, (2,))
        ca1, sa = mod1()
        for i in range(2):
            ln_rows(i * HS // 2, HS // 2, ca1, sa)
            proj_q(i * HS // 2, HS // 2)
        x_b.wait()
        for i in range(2, 4):
            ln_rows(i * HS // 2, HS // 2, ca1, sa)
            proj_q(i * HS // 2, HS // 2)

        zst = pl.multiple_of(z_ref[0], 8)
        zld = pl.multiple_of(z_ref[1], 8)
        dfalse_h = jax.lax.broadcasted_iota(jnp.int32, (R // 2, 128), 1) < z_ref[0]
        seq = [[15], [14, 0], [13, 1], [12, 2], [11, 3], [10, 4], [9, 5], [8, 6], [7]]
        items = [(hh, rs) for hh in range(2) for rs in seq]
        n_items = len(items)
        MAXP = max(len(rs) for rs in seq)

        def attention(p, extra=None):
            pins = {}

            def stage_a(t):
                hh, rs = items[t]
                sb = sbufs[t % NB]
                off = 0
                for pi, r in enumerate(rs):
                    W = R * (r + 1)
                    qu = q_s[hh, r * R // 2:(r + 1) * R // 2, :]
                    if (t - PIN) in pins and pi == 0:
                        for o_prev in pins[t - PIN]:
                            qu = jnp.where(dfalse_h, o_prev, qu)
                    qv = _upk(qu)
                    mx = None
                    for c0 in range(0, W, KC):
                        w = min(KC, W - c0)
                        sc_ = _dot_nt(qv, _upk(k_s[hh, c0 // 2:(c0 + w) // 2, :]))
                        for c1 in range(0, w, 128):
                            tile = sc_[:, c1:c1 + 128]
                            kk = c0 + c1
                            if kk == r * R:
                                tile = jnp.minimum(tile, cap_s[...])
                            sb[pl.ds(zst, R), off + kk:off + kk + 128] = tile
                            mx = tile if mx is None else jnp.maximum(mx, tile)
                    mrow = jnp.max(mx, axis=-1, keepdims=True)
                    mbufs[t % NB][pl.ds(zst, R), pi * 128:(pi + 1) * 128] = jnp.broadcast_to(mrow, (R, 128))
                    off += W

            def stage_f(t):
                hh, rs = items[t]
                sb = sbufs[t % NB]
                off = 0
                pins[t] = []
                for pi, r in enumerate(rs):
                    W = R * (r + 1)
                    mn = mbufs[t % NB][pl.ds(zld, R), pi * 128:(pi + 1) * 128]
                    psum = None
                    pv = None
                    for c0 in range(0, W, KC):
                        w = min(KC, W - c0)
                        prs = []
                        for c1 in range(0, w, 128):
                            kk = off + c0 + c1
                            pr = jnp.exp2(sb[pl.ds(zld, R), kk:kk + 128] - mn)
                            psum = pr if psum is None else psum + pr
                            prs.append(pr)
                        pm = (prs[0] if len(prs) == 1 else jnp.concatenate(prs, axis=1)).astype(BF16)
                        d = _dot(pm, _upk(v_s[hh, c0 // 2:(c0 + w) // 2, :]))
                        pv = d if pv is None else pv + d
                    lt = jnp.sum(psum, axis=-1, keepdims=True)
                    r0_ = pl.reciprocal(lt, approx=True)
                    rl = r0_ * (2.0 - lt * r0_)
                    o = _pk(pv * rl)
                    pins[t].append(o)
                    ctx_s[p, r * R // 2:(r + 1) * R // 2, hh * D:(hh + 1) * D] = o
                    off += W

            for t in range(n_items + 1):
                if t < n_items:
                    stage_a(t)
                if extra is not None and t in extra:
                    extra[t]()
                if t >= 1:
                    stage_f(t - 1)

        def pair_body(p, _):
            nslot = (p + 1) % 2
            for cp in raw_copies(jnp.minimum(p + 2, NP - 1), p % 2):
                cp.start()
            for cp in raw_copies(p + 1, nslot):
                cp.wait()

            def wait_unpack():
                unpack(nslot)
            pieces = []
            for i in range(S // PROJ_RB - 1, -1, -1):
                pieces.append(lambda i=i: proj_q(i * PROJ_RB, PROJ_RB))
                pieces.append(lambda i=i: proj_kv(i * PROJ_RB, PROJ_RB))
            extra = {3: wait_unpack, n_items - 1: pieces[0], n_items: pieces[1]}
            used = 2
            attention(p, extra)
            for f in pieces[used:]:
                f()
            return _

        for cp in late:
            cp.start()
        jax.lax.fori_loop(0, NP - 1, pair_body, None)
        for cp in raw_copies(NP - 1, (NP - 2) % 2):
            cp.wait()
        attention(NP - 1)

        for cp in late:
            cp.wait()
        mod2 = _dot(sc16, wm2_s[...])[0:8].astype(BF16).astype(F32)
        mod_s[...] = mod2

        g_s[0:8, :] = jnp.zeros((8, M), F32)
        g_s[8 + S:16 + S, :] = jnp.zeros((8, M), F32)

        HB1 = EP_RB // EPH

        def ep1_body(r, _):
            halves = []
            for hf in range(EPH):
                r0 = pl.multiple_of(r * EP_RB + hf * HB1, HB1)
                rs = pl.ds(r0, HB1)
                rs2 = pl.ds(pl.multiple_of(r * (EP_RB // 2) + hf * (HB1 // 2), HB1 // 2), HB1 // 2)
                cx = jnp.concatenate([_upk(ctx_s[pp, rs2, :]) for pp in range(NP)], axis=1)
                halves.append((r0, rs, x_s[rs, :], _dot(cx, wo_s[...])))
            ga = mod_s[0:1, 0:M]
            sb_ = mod_s[0:1, M:2 * M]
            cb = mod_s[0:1, 2 * M:3 * M]
            outs = []
            for (r0, rs, xin, acc) in halves:
                x1 = xin.astype(F32) + ga * acc
                hb = _ln(x1) * (1.0 + cb) + sb_
                pre = _dot(_ln(hb).astype(BF16), w1_s[...])
                outs.append((r0, rs, x1, hb, pre))
            for (r0, rs, x1, hb, pre) in outs:
                g = _gelu(pre)
                x1_s[rs, :] = x1
                hb_s[rs, :] = hb
                g_s[pl.ds(r0 + 8, HB1), :] = g
            return _

        HB2 = EP_RB // EPH

        def out_copies(b, slot):
            return [pltpu.make_async_copy(
                o_s.at[slot, pl.ds(hf * HB2, HB2), :],
                out_hbm.at[pl.ds(pl.multiple_of(b * EP_RB + hf * HB2, HB2), HB2), :], osems.at[slot, hf])
                for hf in range(EPH)]


        def ep2_body(r, _):
            @pl.when(r >= 2)
            def _w():
                for cp in out_copies(r - 2, r % 2):
                    cp.wait()
            lane = jax.lax.broadcasted_iota(jnp.int32, (HB2, 128), 1)
            gb = mod_s[0:1, 3 * M:4 * M]
            st1 = []
            for hf in range(EPH):
                r0 = pl.multiple_of(r * EP_RB + hf * HB2, HB2)
                rs = pl.ds(r0, HB2)
                wins = {c0: g_s[pl.ds(r0, HB2 + 16), c0:c0 + 128] for c0 in range(0, M, 128)}
                gm1 = lambda c0: wins[c0][7:7 + HB2]
                gp1 = lambda c0: wins[c0][9:9 + HB2]
                gm2 = lambda c0: wins[c0][6:6 + HB2]
                gp2 = lambda c0: wins[c0][10:10 + HB2]
                t0 = gm1(0)
                t1 = jnp.where(lane < 32, gm1(128), gp1(128))
                t2 = jnp.where(lane < 64, gp1(256), gm2(256))
                t3 = jnp.where(lane < 96, gm2(384), gp2(384))
                t4 = gp2(512)
                gs = jnp.concatenate([t0, t1, t2, t3, t4], axis=1).astype(BF16)
                st1.append((rs, hb_s[rs, :], x1_s[rs, :], _dot(gs, w2_s[...])))
            st2 = []
            for (rs, hbv, x1v, hs) in st1:
                xb = hbv + hs
                u = _gelu(_dot_nt(_ln(xb).astype(BF16), w3_s[...])).astype(BF16)
                st2.append((xb, x1v, u))
            for hf, (xb, x1v, u) in enumerate(st2):
                h2 = _dot(u, w4_s[...])
                o_s[r % 2, hf * HB2:(hf + 1) * HB2, :] = (x1v + gb * (xb + h2)).astype(BF16)
                out_copies(r, r % 2)[hf].start()
            return _

        NE = S // EP_RB
        jax.lax.fori_loop(0, NE, ep1_body, None)
        jax.lax.fori_loop(0, NE, ep2_body, None)
        for r in (NE - 2, NE - 1):
            for cp in out_copies(r, r % 2):
                cp.wait()

    return kernel


def run(A_x, A_c_kv, A_w_q, A_w_uk, A_w_uv, A_w_o, B_x, B_w1, B_w2, B_w3, B_w4, c, w_mod):
    del B_x
    hbm = pl.BlockSpec(memory_space=pltpu.HBM)
    out = pl.pallas_call(
        make_kernel(),
        out_shape=jax.ShapeDtypeStruct((S, M), BF16),
        in_specs=[hbm] * 10 + [pl.BlockSpec(memory_space=pltpu.VMEM), hbm, pl.BlockSpec(memory_space=pltpu.SMEM)],
        out_specs=hbm,
        scratch_shapes=[
            pltpu.VMEM((S, M), BF16), pltpu.VMEM((S, DC), BF16),
            pltpu.VMEM((H * D, M), BF16),
            pltpu.VMEM((M, M), BF16), pltpu.VMEM((M, M), BF16),
            pltpu.VMEM((F, M), BF16), pltpu.VMEM((F, M), BF16),
            pltpu.VMEM((M, 2 * M), BF16), pltpu.VMEM((M, 4 * M), BF16),
            pltpu.VMEM((2, M, D), U32), pltpu.VMEM((2, DC, D), U32), pltpu.VMEM((2, DC, D), U32),
            pltpu.VMEM((M // 2, 2 * D), U32), pltpu.VMEM((DC // 2, 2 * D), U32), pltpu.VMEM((DC // 2, 2 * D), U32),
            pltpu.VMEM((8, 4 * M), F32),
            pltpu.VMEM((S // 2, M), U32),
            pltpu.VMEM((2, S // 2, D), U32), pltpu.VMEM((2, S // 2, D), U32), pltpu.VMEM((2, S // 2, D), U32),
            pltpu.VMEM((NP, S // 2, 2 * D), U32),
            pltpu.VMEM((S, M), F32),
            pltpu.VMEM((S, M), F32),
            pltpu.VMEM((S + 16, M), F32),
            pltpu.VMEM((2, EP_RB, M), BF16),
            pltpu.VMEM((R, 128), F32),
            pltpu.SemaphoreType.DMA((11,)),
            pltpu.SemaphoreType.DMA((2, 3)),
            pltpu.SemaphoreType.DMA((2, EPH)),
        ] + [pltpu.VMEM((R, S), F32)] * NB + [pltpu.VMEM((R, 256), F32)] * NB,
        compiler_params=pltpu.CompilerParams(
            vmem_limit_bytes=120 * 1024 * 1024,
            flags={"XLA_TPU_FORCE_LP_LLO_SCHEDULER": True},
            disable_bounds_checks=True),
    )(A_x.reshape(S, M), A_c_kv.reshape(S, DC), A_w_q, A_w_uk, A_w_uv, A_w_o.reshape(H * D, M),
      B_w1, B_w2, B_w3.T, B_w4, c, w_mod, np.zeros((2,), np.int32))
    return out.reshape(1, S, M)


@jax.jit
def pallas_adaLN_cond__compressed_kv_cla__mixer_s_mlp__prompt_kernel(
    A_x: jax.Array,
    A_c_kv: jax.Array,
    A_w_q: jax.Array,
    A_w_uk: jax.Array,
    A_w_uv: jax.Array,
    A_w_o: jax.Array,
    B_x: jax.Array,
    B_w1: jax.Array,
    B_w2: jax.Array,
    B_w3: jax.Array,
    B_w4: jax.Array,
    c: jax.Array,
    w_mod: jax.Array,
):
    return run(A_x, A_c_kv, A_w_q, A_w_uk, A_w_uv, A_w_o, B_x, B_w1, B_w2, B_w3, B_w4, c, w_mod)
```

```python
import jax
import jax.numpy as jnp
import numpy as np
import jax.experimental.pallas as pl
import jax.experimental.pallas.tpu as pltpu

S = 2048
M = 640
H = 32
D = 128
DC = 512
F = 1728
NP = H // 2
LOG2E = 1.4426950408889634
F32 = jnp.float32
BF16 = jnp.bfloat16
U32 = jnp.uint32


def _ln(x, eps=1e-5):
    m = jnp.mean(x, axis=-1, keepdims=True)
    xc = x - m
    v = jnp.mean(xc * xc, axis=-1, keepdims=True)
    return xc * jax.lax.rsqrt(v + eps)


def _gelu(x):
    return 0.5 * x * (1.0 + jnp.tanh(0.7978845608028654 * (x + 0.044715 * (x * x * x))))


def _dot(a, b):
    return jnp.dot(a, b, preferred_element_type=F32)


def _dot_nt(a, b):
    return jax.lax.dot_general(a, b, (((1,), (1,)), ((), ())), preferred_element_type=F32)


def _pk(x):
    return pltpu.bitcast(x.astype(BF16), U32)


def _upk(u):
    return pltpu.bitcast(u, BF16)


R = 128
KC = 2048
NB = 2
PIN = 3
PROJ_RB = 512
EP_RB = 512
EPH = 4
HS = S // 2


def make_kernel():
    NC = S // R
    qscale = (D ** -0.5) * LOG2E

    def kernel(x_hbm, ckv_hbm, wq_hbm, wuk_hbm, wuv_hbm, wo_hbm, w1_hbm, w2_hbm, w3_hbm, w4_hbm,
               c_ref, wmod_hbm, z_ref, out_hbm,
               x_s, ckv_s, wo_s, w1_s, w2_s, w3_s, w4_s, wm1_s, wm2_s,
               rq_s, rk_s, rv_s, wqp_s, wkp_s, wvp_s,
               mod_s, h_s, q_s, k_s, v_s, ctx_s, x1_s, hb_s, g_s, o_s, cap_s,
               sems, rsems, osems, *bufs):
        sbufs, mbufs = bufs[0:NB], bufs[NB:2 * NB]

        wq_u = wq_hbm.bitcast(U32)
        wuk_u = wuk_hbm.bitcast(U32)
        wuv_u = wuv_hbm.bitcast(U32)

        def raw_copies(p, slot):
            return [pltpu.make_async_copy(wuk_u.at[:, p, :], rk_s.at[slot], rsems.at[slot, 0]),
                    pltpu.make_async_copy(wuv_u.at[:, p, :], rv_s.at[slot], rsems.at[slot, 1]),
                    pltpu.make_async_copy(wq_u.at[:, p, :], rq_s.at[slot], rsems.at[slot, 2])]

        cp_wm1 = pltpu.make_async_copy(wmod_hbm.at[:, 0:2 * M], wm1_s, sems.at[1])
        late = [pltpu.make_async_copy(wmod_hbm.at[:, 2 * M:6 * M], wm2_s, sems.at[3]),
                pltpu.make_async_copy(wo_hbm, wo_s, sems.at[4]),
                pltpu.make_async_copy(w1_hbm, w1_s, sems.at[5]),
                pltpu.make_async_copy(w2_hbm, w2_s, sems.at[6]),
                pltpu.make_async_copy(w3_hbm, w3_s, sems.at[7]),
                pltpu.make_async_copy(w4_hbm, w4_s, sems.at[8])]

        def unpack(slot, which=(0, 1, 2)):
            for (src, dst, rows) in [((rk_s, wkp_s, DC), (rv_s, wvp_s, DC), (rq_s, wqp_s, M))[w_] for w_ in which]:
                CH = 128
                for c0 in range(0, rows, CH):
                    a = src[slot, c0:c0 + CH, :]
                    lo = pltpu.bitcast(a << 16, F32)
                    hi = pltpu.bitcast(a & jnp.uint32(0xFFFF0000), F32)
                    dst[c0 // 2:(c0 + CH) // 2, 0:128] = _pk(lo)
                    dst[c0 // 2:(c0 + CH) // 2, 128:256] = _pk(hi)

        def proj_kv(r0, n):
            ck = ckv_s[pl.ds(r0, n), :]
            k = _dot(ck, _upk(wkp_s[...]))
            v = _dot(ck, _upk(wvp_s[...]))
            h0 = r0 // 2
            for hh in range(2):
                k_s[hh, pl.ds(h0, n // 2), :] = _pk(k[:, hh * D:(hh + 1) * D])
                v_s[hh, pl.ds(h0, n // 2), :] = _pk(v[:, hh * D:(hh + 1) * D])

        def proj_q(r0, n):
            h0 = r0 // 2
            q = _dot(_upk(h_s[pl.ds(h0, n // 2), :]), _upk(wqp_s[...])) * qscale
            for hh in range(2):
                q_s[hh, pl.ds(h0, n // 2), :] = _pk(q[:, hh * D:(hh + 1) * D])

        ri = jax.lax.broadcasted_iota(jnp.int32, (R, 128), 0)
        ci = jax.lax.broadcasted_iota(jnp.int32, (R, 128), 1)
        cap_s[...] = jnp.where(ci <= ri, jnp.finfo(F32).max, -1e9).astype(F32)

        cvec = c_ref[...].astype(F32)
        sc16 = jnp.broadcast_to((cvec * jax.nn.sigmoid(cvec)).astype(BF16), (16, M))

        def ln_rows(r0, n, ca1, sa):
            for a0 in range(r0, r0 + n, 256):
                xb = x_s[a0:a0 + 256, :].astype(F32)
                h_s[a0 // 2:(a0 + 256) // 2, :] = _pk(_ln(xb) * ca1 + sa)

        def mod1():
            m1 = _dot(sc16, wm1_s[...])[0:8].astype(BF16).astype(F32)
            return 1.0 + m1[0:1, M:2 * M], m1[0:1, 0:M]

        raw0 = raw_copies(0, 0)
        ckv_a = pltpu.make_async_copy(ckv_hbm.at[0:HS, :], ckv_s.at[0:HS, :], sems.at[0])
        ckv_b = pltpu.make_async_copy(ckv_hbm.at[HS:S, :], ckv_s.at[HS:S, :], sems.at[9])
        raw0[0].start()
        raw0[1].start()
        ckv_a.start()
        ckv_b.start()
        x_a = pltpu.make_async_copy(x_hbm.at[0:HS, :], x_s.at[0:HS, :], sems.at[2])
        x_b = pltpu.make_async_copy(x_hbm.at[HS:S, :], x_s.at[HS:S, :], sems.at[10])
        raw0[0].wait()
        raw0[1].wait()
        ckv_a.wait()
        cp_wm1.start()
        x_a.start()
        raw0[2].start()
        unpack(0, (0, 1))
        proj_kv(0, HS)
        ckv_b.wait()
        x_b.start()
        for cp in raw_copies(1, 1):
            cp.start()
        proj_kv(HS, HS)
        cp_wm1.wait()
        x_a.wait()
        raw0[2].wait()
        unpack(0, (2,))
        ca1, sa = mod1()
        for i in range(2):
            ln_rows(i * HS // 2, HS // 2, ca1, sa)
            proj_q(i * HS // 2, HS // 2)
        x_b.wait()
        for i in range(2, 4):
            ln_rows(i * HS // 2, HS // 2, ca1, sa)
            proj_q(i * HS // 2, HS // 2)

        zst = pl.multiple_of(z_ref[0], 8)
        zld = pl.multiple_of(z_ref[1], 8)
        dfalse_h = jax.lax.broadcasted_iota(jnp.int32, (R // 2, 128), 1) < z_ref[0]
        seq = [[15],[14,0],[13,1],[12,2],[11,3],[10,4],[9,5],[8,6],[7]]
        items = [(hh, rs) for hh in range(2) for rs in seq]
        n_items = len(items)
        MAXP = max(len(rs) for rs in seq)

        def attention(p, extra=None):
            pins = {}

            def stage_a(t):
                hh, rs = items[t]
                sb = sbufs[t % NB]
                off = 0
                for pi, r in enumerate(rs):
                    W = R * (r + 1)
                    qu = q_s[hh, r * R // 2:(r + 1) * R // 2, :]
                    if (t - PIN) in pins and pi == 0:
                        for o_prev in pins[t - PIN]:
                            qu = jnp.where(dfalse_h, o_prev, qu)
                    qv = _upk(qu)
                    mx = None
                    for c0 in range(0, W, KC):
                        w = min(KC, W - c0)
                        sc_ = _dot_nt(qv, _upk(k_s[hh, c0 // 2:(c0 + w) // 2, :]))
                        for c1 in range(0, w, 128):
                            tile = sc_[:, c1:c1 + 128]
                            kk = c0 + c1
                            if kk == r * R:
                                tile = jnp.minimum(tile, cap_s[...])
                            sb[pl.ds(zst, R), off + kk:off + kk + 128] = tile
                            mx = tile if mx is None else jnp.maximum(mx, tile)
                    mrow = jnp.max(mx, axis=-1, keepdims=True)
                    mbufs[t % NB][pl.ds(zst, R), pi * 128:(pi + 1) * 128] = jnp.broadcast_to(mrow, (R, 128))
                    off += W

            def stage_f(t):
                hh, rs = items[t]
                sb = sbufs[t % NB]
                off = 0
                pins[t] = []
                for pi, r in enumerate(rs):
                    W = R * (r + 1)
                    mn = mbufs[t % NB][pl.ds(zld, R), pi * 128:(pi + 1) * 128]
                    psum = None
                    pv = None
                    for c0 in range(0, W, KC):
                        w = min(KC, W - c0)
                        prs = []
                        for c1 in range(0, w, 128):
                            kk = off + c0 + c1
                            pr = jnp.exp2(sb[pl.ds(zld, R), kk:kk + 128] - mn)
                            psum = pr if psum is None else psum + pr
                            prs.append(pr)
                        pm = (prs[0] if len(prs) == 1 else jnp.concatenate(prs, axis=1)).astype(BF16)
                        d = _dot(pm, _upk(v_s[hh, c0 // 2:(c0 + w) // 2, :]))
                        pv = d if pv is None else pv + d
                    lt = jnp.sum(psum, axis=-1, keepdims=True)
                    r0_ = pl.reciprocal(lt, approx=True)
                    rl = r0_ * (2.0 - lt * r0_)
                    o = _pk(pv * rl)
                    pins[t].append(o)
                    ctx_s[p, r * R // 2:(r + 1) * R // 2, hh * D:(hh + 1) * D] = o
                    off += W

            for t in range(n_items + 1):
                if t < n_items:
                    stage_a(t)
                if extra is not None and t in extra:
                    extra[t]()
                if t >= 1:
                    stage_f(t - 1)

        def pair_body(p, _):
            nslot = (p + 1) % 2
            for cp in raw_copies(p + 1, nslot):
                cp.wait()
            for cp in raw_copies(jnp.minimum(p + 2, NP - 1), p % 2):
                cp.start()

            def wait_unpack():
                unpack(nslot)
            pieces = []
            for i in range(S // PROJ_RB - 1, -1, -1):
                pieces.append(lambda i=i: proj_kv(i * PROJ_RB, PROJ_RB))
                pieces.append(lambda i=i: proj_q(i * PROJ_RB, PROJ_RB))
            extra = {3: wait_unpack, n_items - 1: pieces[0], n_items: pieces[1]}
            used = 2
            attention(p, extra)
            for f in pieces[used:]:
                f()
            return _

        for cp in late:
            cp.start()
        jax.lax.fori_loop(0, NP - 1, pair_body, None)
        for cp in raw_copies(NP - 1, (NP - 2) % 2):
            cp.wait()
        attention(NP - 1)

        for cp in late:
            cp.wait()
        mod2 = _dot(sc16, wm2_s[...])[0:8].astype(BF16).astype(F32)
        mod_s[...] = mod2

        g_s[0:8, :] = jnp.zeros((8, M), F32)
        g_s[8 + S:16 + S, :] = jnp.zeros((8, M), F32)

        HB1 = EP_RB // EPH

        def ep1_body(r, _):
            halves = []
            for hf in range(EPH):
                r0 = pl.multiple_of(r * EP_RB + hf * HB1, HB1)
                rs = pl.ds(r0, HB1)
                rs2 = pl.ds(pl.multiple_of(r * (EP_RB // 2) + hf * (HB1 // 2), HB1 // 2), HB1 // 2)
                cx = jnp.concatenate([_upk(ctx_s[pp, rs2, :]) for pp in range(NP)], axis=1)
                halves.append((r0, rs, x_s[rs, :], _dot(cx, wo_s[...])))
            ga = mod_s[0:1, 0:M]
            sb_ = mod_s[0:1, M:2 * M]
            cb = mod_s[0:1, 2 * M:3 * M]
            outs = []
            for (r0, rs, xin, acc) in halves:
                x1 = xin.astype(F32) + ga * acc
                hb = _ln(x1) * (1.0 + cb) + sb_
                pre = _dot(_ln(hb).astype(BF16), w1_s[...])
                outs.append((r0, rs, x1, hb, pre))
            for (r0, rs, x1, hb, pre) in outs:
                g = _gelu(pre)
                x1_s[rs, :] = x1
                hb_s[rs, :] = hb
                g_s[pl.ds(r0 + 8, HB1), :] = g
            return _

        HB2 = EP_RB // EPH

        def out_copy(b, slot, hf):
            return pltpu.make_async_copy(
                o_s.at[slot, pl.ds(hf * HB2, HB2), :],
                out_hbm.at[pl.ds(pl.multiple_of(b * EP_RB + hf * HB2, HB2), HB2), :], osems.at[slot, hf])


        def ep2_body(r, _):
            @pl.when(r >= 2)
            def _w():
                for hf in range(EPH):
                    out_copy(r - 2, r % 2, hf).wait()
            lane = jax.lax.broadcasted_iota(jnp.int32, (HB2, 128), 1)
            gb = mod_s[0:1, 3 * M:4 * M]
            st1 = []
            for hf in range(EPH):
                r0 = pl.multiple_of(r * EP_RB + hf * HB2, HB2)
                rs = pl.ds(r0, HB2)
                wins = {c0: g_s[pl.ds(r0, HB2 + 16), c0:c0 + 128] for c0 in range(0, M, 128)}
                gm1 = lambda c0: wins[c0][7:7 + HB2]
                gp1 = lambda c0: wins[c0][9:9 + HB2]
                gm2 = lambda c0: wins[c0][6:6 + HB2]
                gp2 = lambda c0: wins[c0][10:10 + HB2]
                t0 = gm1(0)
                t1 = jnp.where(lane < 32, gm1(128), gp1(128))
                t2 = jnp.where(lane < 64, gp1(256), gm2(256))
                t3 = jnp.where(lane < 96, gm2(384), gp2(384))
                t4 = gp2(512)
                gs = jnp.concatenate([t0, t1, t2, t3, t4], axis=1).astype(BF16)
                st1.append((rs, hb_s[rs, :], x1_s[rs, :], _dot(gs, w2_s[...])))
            st2 = []
            for (rs, hbv, x1v, hs) in st1:
                xb = hbv + hs
                u = _gelu(_dot_nt(_ln(xb).astype(BF16), w3_s[...])).astype(BF16)
                st2.append((xb, x1v, u))
            for hf, (xb, x1v, u) in enumerate(st2):
                h2 = _dot(u, w4_s[...])
                o_s[r % 2, hf * HB2:(hf + 1) * HB2, :] = (x1v + gb * (xb + h2)).astype(BF16)
                out_copy(r, r % 2, hf).start()
            return _

        NE = S // EP_RB
        jax.lax.fori_loop(0, NE, ep1_body, None)
        jax.lax.fori_loop(0, NE, ep2_body, None)
        for r in (NE - 2, NE - 1):
            for hf in range(EPH):
                out_copy(r, r % 2, hf).wait()

    return kernel


def run(A_x, A_c_kv, A_w_q, A_w_uk, A_w_uv, A_w_o, B_x, B_w1, B_w2, B_w3, B_w4, c, w_mod):
    del B_x
    hbm = pl.BlockSpec(memory_space=pltpu.HBM)
    out = pl.pallas_call(
        make_kernel(),
        out_shape=jax.ShapeDtypeStruct((S, M), BF16),
        in_specs=[hbm] * 10 + [pl.BlockSpec(memory_space=pltpu.VMEM), hbm, pl.BlockSpec(memory_space=pltpu.SMEM)],
        out_specs=hbm,
        scratch_shapes=[
            pltpu.VMEM((S, M), BF16), pltpu.VMEM((S, DC), BF16),
            pltpu.VMEM((H * D, M), BF16),
            pltpu.VMEM((M, M), BF16), pltpu.VMEM((M, M), BF16),
            pltpu.VMEM((F, M), BF16), pltpu.VMEM((F, M), BF16),
            pltpu.VMEM((M, 2 * M), BF16), pltpu.VMEM((M, 4 * M), BF16),
            pltpu.VMEM((2, M, D), U32), pltpu.VMEM((2, DC, D), U32), pltpu.VMEM((2, DC, D), U32),
            pltpu.VMEM((M // 2, 2 * D), U32), pltpu.VMEM((DC // 2, 2 * D), U32), pltpu.VMEM((DC // 2, 2 * D), U32),
            pltpu.VMEM((8, 4 * M), F32),
            pltpu.VMEM((S // 2, M), U32),
            pltpu.VMEM((2, S // 2, D), U32), pltpu.VMEM((2, S // 2, D), U32), pltpu.VMEM((2, S // 2, D), U32),
            pltpu.VMEM((NP, S // 2, 2 * D), U32),
            pltpu.VMEM((S, M), F32),
            pltpu.VMEM((S, M), F32),
            pltpu.VMEM((S + 16, M), F32),
            pltpu.VMEM((2, EP_RB, M), BF16),
            pltpu.VMEM((R, 128), F32),
            pltpu.SemaphoreType.DMA((11,)),
            pltpu.SemaphoreType.DMA((2, 3)),
            pltpu.SemaphoreType.DMA((2, EPH)),
        ] + [pltpu.VMEM((R, S), F32)] * NB + [pltpu.VMEM((R, 256), F32)] * NB,
        compiler_params=pltpu.CompilerParams(
            vmem_limit_bytes=120 * 1024 * 1024,
            flags={"XLA_TPU_FORCE_LP_LLO_SCHEDULER": True},
            disable_bounds_checks=True),
    )(A_x.reshape(S, M), A_c_kv.reshape(S, DC), A_w_q, A_w_uk, A_w_uv, A_w_o.reshape(H * D, M),
      B_w1, B_w2, B_w3.T, B_w4, c, w_mod, np.zeros((2,), np.int32))
    return out.reshape(1, S, M)


@jax.jit
def pallas_adaLN_cond__compressed_kv_cla__mixer_s_mlp__prompt_kernel(
    A_x: jax.Array,
    A_c_kv: jax.Array,
    A_w_q: jax.Array,
    A_w_uk: jax.Array,
    A_w_uv: jax.Array,
    A_w_o: jax.Array,
    B_x: jax.Array,
    B_w1: jax.Array,
    B_w2: jax.Array,
    B_w3: jax.Array,
    B_w4: jax.Array,
    c: jax.Array,
    w_mod: jax.Array,
):
    return run(A_x, A_c_kv, A_w_q, A_w_uk, A_w_uv, A_w_o, B_x, B_w1, B_w2, B_w3, B_w4, c, w_mod)
```

```python
import jax
import jax.numpy as jnp
import numpy as np
import jax.experimental.pallas as pl
import jax.experimental.pallas.tpu as pltpu

S = 2048
M = 640
H = 32
D = 128
DC = 512
F = 1728
NP = H // 2
LOG2E = 1.4426950408889634
F32 = jnp.float32
BF16 = jnp.bfloat16
U32 = jnp.uint32


def _ln(x, eps=1e-5):
    m = jnp.mean(x, axis=-1, keepdims=True)
    xc = x - m
    v = jnp.mean(xc * xc, axis=-1, keepdims=True)
    return xc * jax.lax.rsqrt(v + eps)


def _gelu(x):
    return 0.5 * x * (1.0 + jnp.tanh(0.7978845608028654 * (x + 0.044715 * (x * x * x))))


def _dot(a, b):
    return jnp.dot(a, b, preferred_element_type=F32)


def _dot_nt(a, b):
    return jax.lax.dot_general(a, b, (((1,), (1,)), ((), ())), preferred_element_type=F32)


def _pk(x):
    return pltpu.bitcast(x.astype(BF16), U32)


def _upk(u):
    return pltpu.bitcast(u, BF16)


R = 128
KC = 2048
NB = 2
PIN = 3
PROJ_RB = 512
EP_RB = 512
EPH = 4
HS = S // 2


def make_kernel():
    NC = S // R
    qscale = (D ** -0.5) * LOG2E

    def kernel(x_hbm, ckv_hbm, wq_hbm, wuk_hbm, wuv_hbm, wo_hbm, w1_hbm, w2_hbm, w3_hbm, w4_hbm,
               c_ref, wmod_hbm, z_ref, out_hbm,
               x_s, ckv_s, wo_s, w1_s, w2_s, w3_s, w4_s, wm1_s, wm2_s,
               rq_s, rk_s, rv_s, wqp_s, wkv_s,
               mod_s, h_s, q_s, k_s, v_s, ctx_s, x1_s, hb_s, g_s, o_s, cap_s,
               sems, rsems, osems, *bufs):
        sbufs, mbufs = bufs[0:NB], bufs[NB:2 * NB]

        wq_u = wq_hbm.bitcast(U32)
        wuk_u = wuk_hbm.bitcast(U32)
        wuv_u = wuv_hbm.bitcast(U32)

        def raw_copies(p, slot):
            return [pltpu.make_async_copy(wuk_u.at[:, p, :], rk_s.at[slot], rsems.at[slot, 0]),
                    pltpu.make_async_copy(wuv_u.at[:, p, :], rv_s.at[slot], rsems.at[slot, 1]),
                    pltpu.make_async_copy(wq_u.at[:, p, :], rq_s.at[slot], rsems.at[slot, 2])]

        cp_wm1 = pltpu.make_async_copy(wmod_hbm.at[:, 0:2 * M], wm1_s, sems.at[1])
        late = [pltpu.make_async_copy(wmod_hbm.at[:, 2 * M:6 * M], wm2_s, sems.at[3]),
                pltpu.make_async_copy(wo_hbm, wo_s, sems.at[4]),
                pltpu.make_async_copy(w1_hbm, w1_s, sems.at[5]),
                pltpu.make_async_copy(w2_hbm, w2_s, sems.at[6]),
                pltpu.make_async_copy(w3_hbm, w3_s, sems.at[7]),
                pltpu.make_async_copy(w4_hbm, w4_s, sems.at[8])]

        def unpack(slot, which=(0, 1, 2)):
            for (src, dst, rows, col) in [((rk_s, wkv_s, DC, 0), (rv_s, wkv_s, DC, 2 * D), (rq_s, wqp_s, M, 0))[w_] for w_ in which]:
                CH = 128
                for c0 in range(0, rows, CH):
                    a = src[slot, c0:c0 + CH, :]
                    lo = pltpu.bitcast(a << 16, F32)
                    hi = pltpu.bitcast(a & jnp.uint32(0xFFFF0000), F32)
                    dst[c0 // 2:(c0 + CH) // 2, col:col + D] = _pk(lo)
                    dst[c0 // 2:(c0 + CH) // 2, col + D:col + 2 * D] = _pk(hi)

        def proj_kv(r0, n):
            kv = _dot(ckv_s[pl.ds(r0, n), :], _upk(wkv_s[...]))
            k, v = kv[:, 0:2 * D], kv[:, 2 * D:4 * D]
            h0 = r0 // 2
            for hh in range(2):
                k_s[hh, pl.ds(h0, n // 2), :] = _pk(k[:, hh * D:(hh + 1) * D])
                v_s[hh, pl.ds(h0, n // 2), :] = _pk(v[:, hh * D:(hh + 1) * D])

        def proj_q(r0, n):
            h0 = r0 // 2
            q = _dot(_upk(h_s[pl.ds(h0, n // 2), :]), _upk(wqp_s[...])) * qscale
            for hh in range(2):
                q_s[hh, pl.ds(h0, n // 2), :] = _pk(q[:, hh * D:(hh + 1) * D])

        ri = jax.lax.broadcasted_iota(jnp.int32, (R, 128), 0)
        ci = jax.lax.broadcasted_iota(jnp.int32, (R, 128), 1)
        cap_s[...] = jnp.where(ci <= ri, jnp.finfo(F32).max, -1e9).astype(F32)

        cvec = c_ref[...].astype(F32)
        sc16 = jnp.broadcast_to((cvec * jax.nn.sigmoid(cvec)).astype(BF16), (16, M))

        def ln_rows(r0, n, ca1, sa):
            for a0 in range(r0, r0 + n, 256):
                xb = x_s[a0:a0 + 256, :].astype(F32)
                h_s[a0 // 2:(a0 + 256) // 2, :] = _pk(_ln(xb) * ca1 + sa)

        def mod1():
            m1 = _dot(sc16, wm1_s[...])[0:8].astype(BF16).astype(F32)
            return 1.0 + m1[0:1, M:2 * M], m1[0:1, 0:M]

        raw0 = raw_copies(0, 0)
        ckv_a = pltpu.make_async_copy(ckv_hbm.at[0:HS, :], ckv_s.at[0:HS, :], sems.at[0])
        ckv_b = pltpu.make_async_copy(ckv_hbm.at[HS:S, :], ckv_s.at[HS:S, :], sems.at[9])
        raw0[0].start()
        raw0[1].start()
        ckv_a.start()
        ckv_b.start()
        x_a = pltpu.make_async_copy(x_hbm.at[0:HS, :], x_s.at[0:HS, :], sems.at[2])
        x_b = pltpu.make_async_copy(x_hbm.at[HS:S, :], x_s.at[HS:S, :], sems.at[10])
        raw0[0].wait()
        raw0[1].wait()
        ckv_a.wait()
        cp_wm1.start()
        x_a.start()
        raw0[2].start()
        unpack(0, (0, 1))
        proj_kv(0, HS)
        ckv_b.wait()
        x_b.start()
        for cp in raw_copies(1, 1):
            cp.start()
        proj_kv(HS, HS)
        cp_wm1.wait()
        x_a.wait()
        raw0[2].wait()
        unpack(0, (2,))
        ca1, sa = mod1()
        for i in range(2):
            ln_rows(i * HS // 2, HS // 2, ca1, sa)
            proj_q(i * HS // 2, HS // 2)
        x_b.wait()
        for i in range(2, 4):
            ln_rows(i * HS // 2, HS // 2, ca1, sa)
            proj_q(i * HS // 2, HS // 2)

        zst = pl.multiple_of(z_ref[0], 8)
        zld = pl.multiple_of(z_ref[1], 8)
        dfalse_h = jax.lax.broadcasted_iota(jnp.int32, (R // 2, 128), 1) < z_ref[0]
        seq = [[15],[14,0],[13,1],[12,2],[11,3],[10,4],[9,5],[8,6],[7]]
        items = [(hh, rs) for hh in range(2) for rs in seq]
        n_items = len(items)
        MAXP = max(len(rs) for rs in seq)

        def attention(p, extra=None):
            pins = {}

            def stage_a(t):
                hh, rs = items[t]
                sb = sbufs[t % NB]
                off = 0
                for pi, r in enumerate(rs):
                    W = R * (r + 1)
                    qu = q_s[hh, r * R // 2:(r + 1) * R // 2, :]
                    if (t - PIN) in pins and pi == 0:
                        for o_prev in pins[t - PIN]:
                            qu = jnp.where(dfalse_h, o_prev, qu)
                    qv = _upk(qu)
                    mx = None
                    for c0 in range(0, W, KC):
                        w = min(KC, W - c0)
                        sc_ = _dot_nt(qv, _upk(k_s[hh, c0 // 2:(c0 + w) // 2, :]))
                        for c1 in range(0, w, 128):
                            tile = sc_[:, c1:c1 + 128]
                            kk = c0 + c1
                            if kk == r * R:
                                tile = jnp.minimum(tile, cap_s[...])
                            sb[pl.ds(zst, R), off + kk:off + kk + 128] = tile
                            mx = tile if mx is None else jnp.maximum(mx, tile)
                    mrow = jnp.max(mx, axis=-1, keepdims=True)
                    mbufs[t % NB][pl.ds(zst, R), pi * 128:(pi + 1) * 128] = jnp.broadcast_to(mrow, (R, 128))
                    off += W

            def stage_f(t):
                hh, rs = items[t]
                sb = sbufs[t % NB]
                off = 0
                pins[t] = []
                for pi, r in enumerate(rs):
                    W = R * (r + 1)
                    mn = mbufs[t % NB][pl.ds(zld, R), pi * 128:(pi + 1) * 128]
                    psum = None
                    pv = None
                    for c0 in range(0, W, KC):
                        w = min(KC, W - c0)
                        prs = []
                        for c1 in range(0, w, 128):
                            kk = off + c0 + c1
                            pr = jnp.exp2(sb[pl.ds(zld, R), kk:kk + 128] - mn)
                            psum = pr if psum is None else psum + pr
                            prs.append(pr)
                        pm = (prs[0] if len(prs) == 1 else jnp.concatenate(prs, axis=1)).astype(BF16)
                        d = _dot(pm, _upk(v_s[hh, c0 // 2:(c0 + w) // 2, :]))
                        pv = d if pv is None else pv + d
                    lt = jnp.sum(psum, axis=-1, keepdims=True)
                    r0_ = pl.reciprocal(lt, approx=True)
                    rl = r0_ * (2.0 - lt * r0_)
                    o = _pk(pv * rl)
                    pins[t].append(o)
                    ctx_s[p, r * R // 2:(r + 1) * R // 2, hh * D:(hh + 1) * D] = o
                    off += W

            for t in range(n_items + 1):
                if t < n_items:
                    stage_a(t)
                if extra is not None and t in extra:
                    extra[t]()
                if t >= 1:
                    stage_f(t - 1)

        def pair_body(p, _):
            nslot = (p + 1) % 2
            for cp in raw_copies(p + 1, nslot):
                cp.wait()
            for cp in raw_copies(jnp.minimum(p + 2, NP - 1), p % 2):
                cp.start()

            def wait_unpack():
                unpack(nslot)
            pieces = []
            for i in range(S // PROJ_RB - 1, -1, -1):
                pieces.append(lambda i=i: proj_kv(i * PROJ_RB, PROJ_RB))
                pieces.append(lambda i=i: proj_q(i * PROJ_RB, PROJ_RB))
            extra = {3: wait_unpack, n_items - 1: pieces[0], n_items: pieces[1]}
            used = 2
            attention(p, extra)
            for f in pieces[used:]:
                f()
            return _

        for cp in late:
            cp.start()
        jax.lax.fori_loop(0, NP - 1, pair_body, None)
        for cp in raw_copies(NP - 1, (NP - 2) % 2):
            cp.wait()
        attention(NP - 1)

        for cp in late:
            cp.wait()
        mod2 = _dot(sc16, wm2_s[...])[0:8].astype(BF16).astype(F32)
        mod_s[...] = mod2

        g_s[0:8, :] = jnp.zeros((8, M), F32)
        g_s[8 + S:16 + S, :] = jnp.zeros((8, M), F32)

        HB1 = EP_RB // 8

        def ep1_body(r, _):
            halves = []
            for hf in range(8):
                r0 = pl.multiple_of(r * EP_RB + hf * HB1, HB1)
                rs = pl.ds(r0, HB1)
                rs2 = pl.ds(pl.multiple_of(r * (EP_RB // 2) + hf * (HB1 // 2), HB1 // 2), HB1 // 2)
                cx = jnp.concatenate([_upk(ctx_s[pp, rs2, :]) for pp in range(NP)], axis=1)
                halves.append((r0, rs, x_s[rs, :], _dot(cx, wo_s[...])))
            ga = mod_s[0:1, 0:M]
            sb_ = mod_s[0:1, M:2 * M]
            cb = mod_s[0:1, 2 * M:3 * M]
            outs = []
            for (r0, rs, xin, acc) in halves:
                x1 = xin.astype(F32) + ga * acc
                hb = _ln(x1) * (1.0 + cb) + sb_
                pre = _dot(_ln(hb).astype(BF16), w1_s[...])
                outs.append((r0, rs, x1, hb, pre))
            for (r0, rs, x1, hb, pre) in outs:
                g = _gelu(pre)
                x1_s[rs, :] = x1
                hb_s[rs, :] = hb
                g_s[pl.ds(r0 + 8, HB1), :] = g
            return _

        HB2 = EP_RB // EPH

        def out_copy(b, slot, hf):
            return pltpu.make_async_copy(
                o_s.at[slot, pl.ds(hf * HB2, HB2), :],
                out_hbm.at[pl.ds(pl.multiple_of(b * EP_RB + hf * HB2, HB2), HB2), :], osems.at[slot, hf])


        def ep2_body(r, _):
            @pl.when(r >= 2)
            def _w():
                for hf in range(EPH):
                    out_copy(r - 2, r % 2, hf).wait()
            lane = jax.lax.broadcasted_iota(jnp.int32, (HB2, 128), 1)
            gb = mod_s[0:1, 3 * M:4 * M]
            st1 = []
            for hf in range(EPH):
                r0 = pl.multiple_of(r * EP_RB + hf * HB2, HB2)
                rs = pl.ds(r0, HB2)
                wins = {c0: g_s[pl.ds(r0, HB2 + 16), c0:c0 + 128] for c0 in range(0, M, 128)}
                gm1 = lambda c0: wins[c0][7:7 + HB2]
                gp1 = lambda c0: wins[c0][9:9 + HB2]
                gm2 = lambda c0: wins[c0][6:6 + HB2]
                gp2 = lambda c0: wins[c0][10:10 + HB2]
                t0 = gm1(0)
                t1 = jnp.where(lane < 32, gm1(128), gp1(128))
                t2 = jnp.where(lane < 64, gp1(256), gm2(256))
                t3 = jnp.where(lane < 96, gm2(384), gp2(384))
                t4 = gp2(512)
                gs = jnp.concatenate([t0, t1, t2, t3, t4], axis=1).astype(BF16)
                st1.append((rs, hb_s[rs, :], x1_s[rs, :], _dot(gs, w2_s[...])))
            st2 = []
            for (rs, hbv, x1v, hs) in st1:
                xb = hbv + hs
                u = _gelu(_dot_nt(_ln(xb).astype(BF16), w3_s[...])).astype(BF16)
                st2.append((xb, x1v, u))
            for hf, (xb, x1v, u) in enumerate(st2):
                h2 = _dot(u, w4_s[...])
                o_s[r % 2, hf * HB2:(hf + 1) * HB2, :] = (x1v + gb * (xb + h2)).astype(BF16)
                out_copy(r, r % 2, hf).start()
            return _

        NE = S // EP_RB
        jax.lax.fori_loop(0, NE, ep1_body, None)
        jax.lax.fori_loop(0, NE, ep2_body, None)
        for r in (NE - 2, NE - 1):
            for hf in range(EPH):
                out_copy(r, r % 2, hf).wait()

    return kernel


def run(A_x, A_c_kv, A_w_q, A_w_uk, A_w_uv, A_w_o, B_x, B_w1, B_w2, B_w3, B_w4, c, w_mod):
    del B_x
    hbm = pl.BlockSpec(memory_space=pltpu.HBM)
    out = pl.pallas_call(
        make_kernel(),
        out_shape=jax.ShapeDtypeStruct((S, M), BF16),
        in_specs=[hbm] * 10 + [pl.BlockSpec(memory_space=pltpu.VMEM), hbm, pl.BlockSpec(memory_space=pltpu.SMEM)],
        out_specs=hbm,
        scratch_shapes=[
            pltpu.VMEM((S, M), BF16), pltpu.VMEM((S, DC), BF16),
            pltpu.VMEM((H * D, M), BF16),
            pltpu.VMEM((M, M), BF16), pltpu.VMEM((M, M), BF16),
            pltpu.VMEM((F, M), BF16), pltpu.VMEM((F, M), BF16),
            pltpu.VMEM((M, 2 * M), BF16), pltpu.VMEM((M, 4 * M), BF16),
            pltpu.VMEM((2, M, D), U32), pltpu.VMEM((2, DC, D), U32), pltpu.VMEM((2, DC, D), U32),
            pltpu.VMEM((M // 2, 2 * D), U32), pltpu.VMEM((DC // 2, 4 * D), U32),
            pltpu.VMEM((8, 4 * M), F32),
            pltpu.VMEM((S // 2, M), U32),
            pltpu.VMEM((2, S // 2, D), U32), pltpu.VMEM((2, S // 2, D), U32), pltpu.VMEM((2, S // 2, D), U32),
            pltpu.VMEM((NP, S // 2, 2 * D), U32),
            pltpu.VMEM((S, M), F32),
            pltpu.VMEM((S, M), F32),
            pltpu.VMEM((S + 16, M), F32),
            pltpu.VMEM((2, EP_RB, M), BF16),
            pltpu.VMEM((R, 128), F32),
            pltpu.SemaphoreType.DMA((11,)),
            pltpu.SemaphoreType.DMA((2, 3)),
            pltpu.SemaphoreType.DMA((2, EPH)),
        ] + [pltpu.VMEM((R, S), F32)] * NB + [pltpu.VMEM((R, 256), F32)] * NB,
        compiler_params=pltpu.CompilerParams(
            vmem_limit_bytes=120 * 1024 * 1024,
            flags={"XLA_TPU_FORCE_LP_LLO_SCHEDULER": True},
            disable_bounds_checks=True),
    )(A_x.reshape(S, M), A_c_kv.reshape(S, DC), A_w_q, A_w_uk, A_w_uv, A_w_o.reshape(H * D, M),
      B_w1, B_w2, B_w3.T, B_w4, c, w_mod, np.zeros((2,), np.int32))
    return out.reshape(1, S, M)


@jax.jit
def pallas_adaLN_cond__compressed_kv_cla__mixer_s_mlp__prompt_kernel(
    A_x: jax.Array,
    A_c_kv: jax.Array,
    A_w_q: jax.Array,
    A_w_uk: jax.Array,
    A_w_uv: jax.Array,
    A_w_o: jax.Array,
    B_x: jax.Array,
    B_w1: jax.Array,
    B_w2: jax.Array,
    B_w3: jax.Array,
    B_w4: jax.Array,
    c: jax.Array,
    w_mod: jax.Array,
):
    return run(A_x, A_c_kv, A_w_q, A_w_uk, A_w_uv, A_w_o, B_x, B_w1, B_w2, B_w3, B_w4, c, w_mod)
```

```python
import jax
import jax.numpy as jnp
import numpy as np
import jax.experimental.pallas as pl
import jax.experimental.pallas.tpu as pltpu

S = 2048
M = 640
H = 32
D = 128
DC = 512
F = 1728
NP = H // 2
LOG2E = 1.4426950408889634
F32 = jnp.float32
BF16 = jnp.bfloat16
U32 = jnp.uint32


def _ln(x, eps=1e-5):
    m = jnp.mean(x, axis=-1, keepdims=True)
    xc = x - m
    v = jnp.mean(xc * xc, axis=-1, keepdims=True)
    return xc * jax.lax.rsqrt(v + eps)


def _gelu(x):
    return 0.5 * x * (1.0 + jnp.tanh(0.7978845608028654 * (x + 0.044715 * (x * x * x))))


def _dot(a, b):
    return jnp.dot(a, b, preferred_element_type=F32)


def _dot_nt(a, b):
    return jax.lax.dot_general(a, b, (((1,), (1,)), ((), ())), preferred_element_type=F32)


def _pk(x):
    return pltpu.bitcast(x.astype(BF16), U32)


def _upk(u):
    return pltpu.bitcast(u, BF16)


R = 128
KC = 2048
NB = 2
PIN = 3
PROJ_RB = 512
EP_RB = 512
EPH1 = 8
EPH = 4
HS = S // 2


def make_kernel():
    qscale = (D ** -0.5) * LOG2E

    def kernel(x_hbm, ckv_hbm, wq_hbm, wuk_hbm, wuv_hbm, wo_hbm, w1_hbm, w2_hbm, w3_hbm, w4_hbm,
               c_ref, wmod_hbm, z_ref, out_hbm,
               x_s, ckv_s, wo_s, w1_s, w2_s, w3_s, w4_s, wm1_s, wm2_s,
               rq_s, rk_s, rv_s, wqp_s, wkv_s,
               mod_s, h_s, q_s, k_s, v_s, ctx_s, x1_s, hb_s, g_s, o_s, cap_s,
               sems, rsems, osems, *bufs):
        sbufs, mbufs = bufs[0:NB], bufs[NB:2 * NB]

        wq_u = wq_hbm.bitcast(U32)
        wuk_u = wuk_hbm.bitcast(U32)
        wuv_u = wuv_hbm.bitcast(U32)

        def raw_copies(p, slot):
            return [pltpu.make_async_copy(wuk_u.at[:, p, :], rk_s.at[slot], rsems.at[slot, 0]),
                    pltpu.make_async_copy(wuv_u.at[:, p, :], rv_s.at[slot], rsems.at[slot, 1]),
                    pltpu.make_async_copy(wq_u.at[:, p, :], rq_s.at[slot], rsems.at[slot, 2])]

        cp_wm1 = pltpu.make_async_copy(wmod_hbm.at[:, 0:2 * M], wm1_s, sems.at[1])
        late = [pltpu.make_async_copy(wmod_hbm.at[:, 2 * M:6 * M], wm2_s, sems.at[3]),
                pltpu.make_async_copy(wo_hbm, wo_s, sems.at[4]),
                pltpu.make_async_copy(w1_hbm, w1_s, sems.at[5]),
                pltpu.make_async_copy(w2_hbm, w2_s, sems.at[6]),
                pltpu.make_async_copy(w3_hbm, w3_s, sems.at[7]),
                pltpu.make_async_copy(w4_hbm, w4_s, sems.at[8])]

        def unpack(slot, which=(0, 1, 2)):
            for (src, dst, rows, col) in [((rk_s, wkv_s, DC, 0), (rv_s, wkv_s, DC, 2 * D), (rq_s, wqp_s, M, 0))[w_] for w_ in which]:
                CH = 128
                for c0 in range(0, rows, CH):
                    a = src[slot, c0:c0 + CH, :]
                    lo = pltpu.bitcast(a << 16, F32)
                    hi = pltpu.bitcast(a & jnp.uint32(0xFFFF0000), F32)
                    dst[c0 // 2:(c0 + CH) // 2, col:col + D] = _pk(lo)
                    dst[c0 // 2:(c0 + CH) // 2, col + D:col + 2 * D] = _pk(hi)

        def proj_kv(r0, n):
            kv = _dot(ckv_s[pl.ds(r0, n), :], _upk(wkv_s[...]))
            k, v = kv[:, 0:2 * D], kv[:, 2 * D:4 * D]
            h0 = r0 // 2
            for hh in range(2):
                k_s[hh, pl.ds(h0, n // 2), :] = _pk(k[:, hh * D:(hh + 1) * D])
                v_s[hh, pl.ds(h0, n // 2), :] = _pk(v[:, hh * D:(hh + 1) * D])

        def proj_q(r0, n):
            h0 = r0 // 2
            q = _dot(_upk(h_s[pl.ds(h0, n // 2), :]), _upk(wqp_s[...])) * qscale
            for hh in range(2):
                q_s[hh, pl.ds(h0, n // 2), :] = _pk(q[:, hh * D:(hh + 1) * D])

        ri = jax.lax.broadcasted_iota(jnp.int32, (R, 128), 0)
        ci = jax.lax.broadcasted_iota(jnp.int32, (R, 128), 1)
        cap_s[...] = jnp.where(ci <= ri, jnp.finfo(F32).max, -1e9).astype(F32)

        cvec = c_ref[...].astype(F32)
        sc16 = jnp.broadcast_to((cvec * jax.nn.sigmoid(cvec)).astype(BF16), (16, M))

        def ln_rows(r0, n, ca1, sa):
            for a0 in range(r0, r0 + n, 256):
                xb = x_s[a0:a0 + 256, :].astype(F32)
                h_s[a0 // 2:(a0 + 256) // 2, :] = _pk(_ln(xb) * ca1 + sa)

        def mod1():
            m1 = _dot(sc16, wm1_s[...])[0:8].astype(BF16).astype(F32)
            return 1.0 + m1[0:1, M:2 * M], m1[0:1, 0:M]

        raw0 = raw_copies(0, 0)
        ckv_a = pltpu.make_async_copy(ckv_hbm.at[0:HS, :], ckv_s.at[0:HS, :], sems.at[0])
        ckv_b = pltpu.make_async_copy(ckv_hbm.at[HS:S, :], ckv_s.at[HS:S, :], sems.at[9])
        raw0[0].start()
        raw0[1].start()
        ckv_a.start()
        ckv_b.start()
        x_a = pltpu.make_async_copy(x_hbm.at[0:HS, :], x_s.at[0:HS, :], sems.at[2])
        x_b = pltpu.make_async_copy(x_hbm.at[HS:S, :], x_s.at[HS:S, :], sems.at[10])
        raw0[0].wait()
        raw0[1].wait()
        ckv_a.wait()
        cp_wm1.start()
        x_a.start()
        raw0[2].start()
        unpack(0, (0, 1))
        proj_kv(0, HS)
        ckv_b.wait()
        x_b.start()
        for cp in raw_copies(1, 1):
            cp.start()
        proj_kv(HS, HS)
        cp_wm1.wait()
        x_a.wait()
        raw0[2].wait()
        unpack(0, (2,))
        ca1, sa = mod1()
        for i in range(2):
            ln_rows(i * HS // 2, HS // 2, ca1, sa)
            proj_q(i * HS // 2, HS // 2)
        x_b.wait()
        for i in range(2, 4):
            ln_rows(i * HS // 2, HS // 2, ca1, sa)
            proj_q(i * HS // 2, HS // 2)

        zld = pl.multiple_of(z_ref[0], 8)
        dfalse_h = jax.lax.broadcasted_iota(jnp.int32, (R // 2, 128), 1) < z_ref[0]
        seq = [[15], [14, 0], [13, 1], [12, 2], [11, 3], [10, 4], [9, 5], [8, 6], [7]]
        items = [(hh, rs) for hh in range(2) for rs in seq]
        n_items = len(items)

        def attention(p, extra=None):
            pins = {}

            def stage_a(t):
                hh, rs = items[t]
                sb = sbufs[t % NB]
                off = 0
                for pi, r in enumerate(rs):
                    W = R * (r + 1)
                    qu = q_s[hh, r * R // 2:(r + 1) * R // 2, :]
                    if (t - PIN) in pins and pi == 0:
                        for o_prev in pins[t - PIN]:
                            qu = jnp.where(dfalse_h, o_prev, qu)
                    qv = _upk(qu)
                    mx = None
                    for c0 in range(0, W, KC):
                        w = min(KC, W - c0)
                        sc_ = _dot_nt(qv, _upk(k_s[hh, c0 // 2:(c0 + w) // 2, :]))
                        for c1 in range(0, w, 128):
                            tile = sc_[:, c1:c1 + 128]
                            kk = c0 + c1
                            if kk == r * R:
                                tile = jnp.minimum(tile, cap_s[...])
                            sb[:, off + kk:off + kk + 128] = tile
                            mx = tile if mx is None else jnp.maximum(mx, tile)
                    mrow = jnp.max(mx, axis=-1, keepdims=True)
                    mbufs[t % NB][:, pi * 128:(pi + 1) * 128] = jnp.broadcast_to(mrow, (R, 128))
                    off += W

            def stage_f(t):
                hh, rs = items[t]
                sb = sbufs[t % NB]
                off = 0
                pins[t] = []
                for pi, r in enumerate(rs):
                    W = R * (r + 1)
                    mn = mbufs[t % NB][pl.ds(zld, R), pi * 128:(pi + 1) * 128]
                    psum = None
                    pv = None
                    for c0 in range(0, W, KC):
                        w = min(KC, W - c0)
                        prs = []
                        for c1 in range(0, w, 128):
                            kk = off + c0 + c1
                            pr = jnp.exp2(sb[pl.ds(zld, R), kk:kk + 128] - mn)
                            psum = pr if psum is None else psum + pr
                            prs.append(pr)
                        pm = (prs[0] if len(prs) == 1 else jnp.concatenate(prs, axis=1)).astype(BF16)
                        d = _dot(pm, _upk(v_s[hh, c0 // 2:(c0 + w) // 2, :]))
                        pv = d if pv is None else pv + d
                    lt = jnp.sum(psum, axis=-1, keepdims=True)
                    r0_ = pl.reciprocal(lt, approx=True)
                    rl = r0_ * (2.0 - lt * r0_)
                    o = _pk(pv * rl)
                    pins[t].append(o)
                    ctx_s[p, r * R // 2:(r + 1) * R // 2, hh * D:(hh + 1) * D] = o
                    off += W

            for t in range(n_items + 1):
                if t < n_items:
                    stage_a(t)
                if extra is not None and t in extra:
                    extra[t]()
                if t >= 1:
                    stage_f(t - 1)

        def pair_body(p, _):
            nslot = (p + 1) % 2
            for cp in raw_copies(p + 1, nslot):
                cp.wait()
            for cp in raw_copies(jnp.minimum(p + 2, NP - 1), p % 2):
                cp.start()

            def wait_unpack():
                unpack(nslot)
            pieces = []
            for i in range(S // PROJ_RB - 1, -1, -1):
                pieces.append(lambda i=i: proj_kv(i * PROJ_RB, PROJ_RB))
                pieces.append(lambda i=i: proj_q(i * PROJ_RB, PROJ_RB))
            extra = {3: wait_unpack, n_items - 1: pieces[0], n_items: pieces[1]}
            used = 2
            attention(p, extra)
            for f in pieces[used:]:
                f()
            return _

        for cp in late:
            cp.start()
        jax.lax.fori_loop(0, NP - 1, pair_body, None)
        for cp in raw_copies(NP - 1, (NP - 2) % 2):
            cp.wait()
        attention(NP - 1)

        for cp in late:
            cp.wait()
        mod2 = _dot(sc16, wm2_s[...])[0:8].astype(BF16).astype(F32)
        mod_s[...] = mod2

        g_s[0:8, :] = jnp.zeros((8, M), F32)
        g_s[8 + S:16 + S, :] = jnp.zeros((8, M), F32)

        HB1 = EP_RB // EPH1

        def ep1_body(r, _):
            halves = []
            for hf in range(EPH1):
                r0 = pl.multiple_of(r * EP_RB + hf * HB1, HB1)
                rs = pl.ds(r0, HB1)
                rs2 = pl.ds(pl.multiple_of(r * (EP_RB // 2) + hf * (HB1 // 2), HB1 // 2), HB1 // 2)
                cx = jnp.concatenate([_upk(ctx_s[pp, rs2, :]) for pp in range(NP)], axis=1)
                halves.append((r0, rs, x_s[rs, :], _dot(cx, wo_s[...])))
            ga = mod_s[0:1, 0:M]
            sb_ = mod_s[0:1, M:2 * M]
            cb = mod_s[0:1, 2 * M:3 * M]
            outs = []
            for (r0, rs, xin, acc) in halves:
                x1 = xin.astype(F32) + ga * acc
                hb = _ln(x1) * (1.0 + cb) + sb_
                pre = _dot(_ln(hb).astype(BF16), w1_s[...])
                outs.append((r0, rs, x1, hb, pre))
            for (r0, rs, x1, hb, pre) in outs:
                g = _gelu(pre)
                x1_s[rs, :] = x1
                hb_s[rs, :] = hb
                g_s[pl.ds(r0 + 8, HB1), :] = g
            return _

        HB2 = EP_RB // EPH

        def out_copy(b, slot, hf):
            return pltpu.make_async_copy(
                o_s.at[slot, pl.ds(hf * HB2, HB2), :],
                out_hbm.at[pl.ds(pl.multiple_of(b * EP_RB + hf * HB2, HB2), HB2), :], osems.at[slot, hf])


        def ep2_body(r, _):
            @pl.when(r >= 2)
            def _w():
                for hf in range(EPH):
                    out_copy(r - 2, r % 2, hf).wait()
            lane = jax.lax.broadcasted_iota(jnp.int32, (HB2, 128), 1)
            gb = mod_s[0:1, 3 * M:4 * M]
            st1 = []
            for hf in range(EPH):
                r0 = pl.multiple_of(r * EP_RB + hf * HB2, HB2)
                rs = pl.ds(r0, HB2)
                wins = {c0: g_s[pl.ds(r0, HB2 + 16), c0:c0 + 128] for c0 in range(0, M, 128)}
                gm1 = lambda c0: wins[c0][7:7 + HB2]
                gp1 = lambda c0: wins[c0][9:9 + HB2]
                gm2 = lambda c0: wins[c0][6:6 + HB2]
                gp2 = lambda c0: wins[c0][10:10 + HB2]
                t0 = gm1(0)
                t1 = jnp.where(lane < 32, gm1(128), gp1(128))
                t2 = jnp.where(lane < 64, gp1(256), gm2(256))
                t3 = jnp.where(lane < 96, gm2(384), gp2(384))
                t4 = gp2(512)
                gs = jnp.concatenate([t0, t1, t2, t3, t4], axis=1).astype(BF16)
                st1.append((rs, hb_s[rs, :], x1_s[rs, :], _dot(gs, w2_s[...])))
            st2 = []
            for (rs, hbv, x1v, hs) in st1:
                xb = hbv + hs
                u = _gelu(_dot_nt(_ln(xb).astype(BF16), w3_s[...])).astype(BF16)
                st2.append((xb, x1v, u))
            for hf, (xb, x1v, u) in enumerate(st2):
                h2 = _dot(u, w4_s[...])
                o_s[r % 2, hf * HB2:(hf + 1) * HB2, :] = (x1v + gb * (xb + h2)).astype(BF16)
                out_copy(r, r % 2, hf).start()
            return _

        NE = S // EP_RB
        jax.lax.fori_loop(0, NE, ep1_body, None)
        jax.lax.fori_loop(0, NE, ep2_body, None)
        for r in (NE - 2, NE - 1):
            for hf in range(EPH):
                out_copy(r, r % 2, hf).wait()

    return kernel


def run(A_x, A_c_kv, A_w_q, A_w_uk, A_w_uv, A_w_o, B_x, B_w1, B_w2, B_w3, B_w4, c, w_mod):
    del B_x
    hbm = pl.BlockSpec(memory_space=pltpu.HBM)
    out = pl.pallas_call(
        make_kernel(),
        out_shape=jax.ShapeDtypeStruct((S, M), BF16),
        in_specs=[hbm] * 10 + [pl.BlockSpec(memory_space=pltpu.VMEM), hbm, pl.BlockSpec(memory_space=pltpu.SMEM)],
        out_specs=hbm,
        scratch_shapes=[
            pltpu.VMEM((S, M), BF16), pltpu.VMEM((S, DC), BF16),
            pltpu.VMEM((H * D, M), BF16),
            pltpu.VMEM((M, M), BF16), pltpu.VMEM((M, M), BF16),
            pltpu.VMEM((F, M), BF16), pltpu.VMEM((F, M), BF16),
            pltpu.VMEM((M, 2 * M), BF16), pltpu.VMEM((M, 4 * M), BF16),
            pltpu.VMEM((2, M, D), U32), pltpu.VMEM((2, DC, D), U32), pltpu.VMEM((2, DC, D), U32),
            pltpu.VMEM((M // 2, 2 * D), U32), pltpu.VMEM((DC // 2, 4 * D), U32),
            pltpu.VMEM((8, 4 * M), F32),
            pltpu.VMEM((S // 2, M), U32),
            pltpu.VMEM((2, S // 2, D), U32), pltpu.VMEM((2, S // 2, D), U32), pltpu.VMEM((2, S // 2, D), U32),
            pltpu.VMEM((NP, S // 2, 2 * D), U32),
            pltpu.VMEM((S, M), F32),
            pltpu.VMEM((S, M), F32),
            pltpu.VMEM((S + 16, M), F32),
            pltpu.VMEM((2, EP_RB, M), BF16),
            pltpu.VMEM((R, 128), F32),
            pltpu.SemaphoreType.DMA((11,)),
            pltpu.SemaphoreType.DMA((2, 3)),
            pltpu.SemaphoreType.DMA((2, EPH)),
        ] + [pltpu.VMEM((R, S), F32)] * NB + [pltpu.VMEM((R, 256), F32)] * NB,
        compiler_params=pltpu.CompilerParams(
            vmem_limit_bytes=120 * 1024 * 1024,
            flags={"XLA_TPU_FORCE_LP_LLO_SCHEDULER": True},
            disable_bounds_checks=True),
    )(A_x.reshape(S, M), A_c_kv.reshape(S, DC), A_w_q, A_w_uk, A_w_uv, A_w_o.reshape(H * D, M),
      B_w1, B_w2, B_w3.T, B_w4, c, w_mod, np.zeros((1,), np.int32))
    return out.reshape(1, S, M)


@jax.jit
def pallas_adaLN_cond__compressed_kv_cla__mixer_s_mlp__prompt_kernel(
    A_x: jax.Array,
    A_c_kv: jax.Array,
    A_w_q: jax.Array,
    A_w_uk: jax.Array,
    A_w_uv: jax.Array,
    A_w_o: jax.Array,
    B_x: jax.Array,
    B_w1: jax.Array,
    B_w2: jax.Array,
    B_w3: jax.Array,
    B_w4: jax.Array,
    c: jax.Array,
    w_mod: jax.Array,
):
    return run(A_x, A_c_kv, A_w_q, A_w_uk, A_w_uv, A_w_o, B_x, B_w1, B_w2, B_w3, B_w4, c, w_mod)
```

```python
import jax
import jax.numpy as jnp
import numpy as np
import jax.experimental.pallas as pl
import jax.experimental.pallas.tpu as pltpu

S = 2048
M = 640
H = 32
D = 128
DC = 512
F = 1728
NP = H // 2
LOG2E = 1.4426950408889634
F32 = jnp.float32
BF16 = jnp.bfloat16
U32 = jnp.uint32


def _ln(x, eps=1e-5):
    m = jnp.mean(x, axis=-1, keepdims=True)
    xc = x - m
    v = jnp.mean(xc * xc, axis=-1, keepdims=True)
    return xc * jax.lax.rsqrt(v + eps)


def _gelu(x):
    return 0.5 * x * (1.0 + jnp.tanh(0.7978845608028654 * (x + 0.044715 * (x * x * x))))


def _dot(a, b):
    return jnp.dot(a, b, preferred_element_type=F32)


def _dot_nt(a, b):
    return jax.lax.dot_general(a, b, (((1,), (1,)), ((), ())), preferred_element_type=F32)


def _pk(x):
    return pltpu.bitcast(x.astype(BF16), U32)


def _upk(u):
    return pltpu.bitcast(u, BF16)


R = 128
KC = 2048
NB = 2
PIN = 3
PROJ_RB = 512
EP_RB = 512
EPH1 = 8
EPH = 4
HS = S // 2


def make_kernel():
    qscale = (D ** -0.5) * LOG2E

    def kernel(x_hbm, ckv_hbm, wq_hbm, wuk_hbm, wuv_hbm, wo_hbm, w1_hbm, w2_hbm, w3_hbm, w4_hbm,
               c_ref, wmod_hbm, z_ref, out_hbm,
               x_s, ckv_s, wo_s, w1_s, w2_s, w3_s, w4_s, wm1_s, wm2_s,
               rq_s, rk_s, rv_s, wqp_s, wkv_s,
               mod_s, h_s, q_s, k_s, v_s, ctx_s, x1_s, hb_s, g_s, o_s, cap_s,
               sems, rsems, osems, *bufs):
        sbufs, mbufs = bufs[0:NB], bufs[NB:2 * NB]

        wq_u = wq_hbm.bitcast(U32)
        wuk_u = wuk_hbm.bitcast(U32)
        wuv_u = wuv_hbm.bitcast(U32)

        def raw_copies(p, slot):
            return [pltpu.make_async_copy(wuk_u.at[:, p, :], rk_s.at[slot], rsems.at[slot, 0]),
                    pltpu.make_async_copy(wuv_u.at[:, p, :], rv_s.at[slot], rsems.at[slot, 1]),
                    pltpu.make_async_copy(wq_u.at[:, p, :], rq_s.at[slot], rsems.at[slot, 2])]

        cp_wm1 = pltpu.make_async_copy(wmod_hbm.at[:, 0:2 * M], wm1_s, sems.at[1])
        late = [pltpu.make_async_copy(wmod_hbm.at[:, 2 * M:6 * M], wm2_s, sems.at[3]),
                pltpu.make_async_copy(wo_hbm, wo_s, sems.at[4]),
                pltpu.make_async_copy(w1_hbm, w1_s, sems.at[5]),
                pltpu.make_async_copy(w2_hbm, w2_s, sems.at[6]),
                pltpu.make_async_copy(w3_hbm, w3_s, sems.at[7]),
                pltpu.make_async_copy(w4_hbm, w4_s, sems.at[8])]

        def unpack(slot, which=(0, 1, 2)):
            for (src, dst, rows, col) in [((rk_s, wkv_s, DC, 0), (rv_s, wkv_s, DC, 2 * D), (rq_s, wqp_s, M, 0))[w_] for w_ in which]:
                CH = 128
                for c0 in range(0, rows, CH):
                    a = src[slot, c0:c0 + CH, :]
                    lo = pltpu.bitcast(a << 16, F32)
                    hi = pltpu.bitcast(a & jnp.uint32(0xFFFF0000), F32)
                    dst[c0 // 2:(c0 + CH) // 2, col:col + D] = _pk(lo)
                    dst[c0 // 2:(c0 + CH) // 2, col + D:col + 2 * D] = _pk(hi)

        def proj_kv(r0, n):
            kv = _dot(ckv_s[pl.ds(r0, n), :], _upk(wkv_s[...]))
            k, v = kv[:, 0:2 * D], kv[:, 2 * D:4 * D]
            h0 = r0 // 2
            for hh in range(2):
                k_s[hh, pl.ds(h0, n // 2), :] = _pk(k[:, hh * D:(hh + 1) * D])
                v_s[hh, pl.ds(h0, n // 2), :] = _pk(v[:, hh * D:(hh + 1) * D])

        def proj_q(r0, n):
            h0 = r0 // 2
            q = _dot(_upk(h_s[pl.ds(h0, n // 2), :]), _upk(wqp_s[...])) * qscale
            for hh in range(2):
                q_s[hh, pl.ds(h0, n // 2), :] = _pk(q[:, hh * D:(hh + 1) * D])

        ri = jax.lax.broadcasted_iota(jnp.int32, (R, 128), 0)
        ci = jax.lax.broadcasted_iota(jnp.int32, (R, 128), 1)
        cap_s[...] = jnp.where(ci <= ri, jnp.finfo(F32).max, -1e9).astype(F32)

        cvec = c_ref[...].astype(F32)
        sc16 = jnp.broadcast_to((cvec * jax.nn.sigmoid(cvec)).astype(BF16), (16, M))

        def ln_rows(r0, n, ca1, sa):
            for a0 in range(r0, r0 + n, 256):
                xb = x_s[a0:a0 + 256, :].astype(F32)
                h_s[a0 // 2:(a0 + 256) // 2, :] = _pk(_ln(xb) * ca1 + sa)

        def mod1():
            m1 = _dot(sc16, wm1_s[...])[0:8].astype(BF16).astype(F32)
            return 1.0 + m1[0:1, M:2 * M], m1[0:1, 0:M]

        raw0 = raw_copies(0, 0)
        ckv_a = pltpu.make_async_copy(ckv_hbm.at[0:HS, :], ckv_s.at[0:HS, :], sems.at[0])
        ckv_b = pltpu.make_async_copy(ckv_hbm.at[HS:S, :], ckv_s.at[HS:S, :], sems.at[9])
        raw0[0].start()
        raw0[1].start()
        ckv_a.start()
        ckv_b.start()
        x_a = pltpu.make_async_copy(x_hbm.at[0:HS, :], x_s.at[0:HS, :], sems.at[2])
        x_b = pltpu.make_async_copy(x_hbm.at[HS:S, :], x_s.at[HS:S, :], sems.at[10])
        raw0[0].wait()
        raw0[1].wait()
        ckv_a.wait()
        cp_wm1.start()
        x_a.start()
        raw0[2].start()
        unpack(0, (0, 1))
        proj_kv(0, HS)
        ckv_b.wait()
        x_b.start()
        for cp in raw_copies(1, 1):
            cp.start()
        proj_kv(HS, HS)
        cp_wm1.wait()
        x_a.wait()
        raw0[2].wait()
        unpack(0, (2,))
        ca1, sa = mod1()
        LB = 256
        for half in range(2):
            if half == 1:
                x_b.wait()
            ln_rows(half * HS, LB, ca1, sa)
            for r0 in range(half * HS, (half + 1) * HS, LB):
                if r0 + LB < (half + 1) * HS:
                    ln_rows(r0 + LB, LB, ca1, sa)
                proj_q(r0, LB)

        zld = pl.multiple_of(z_ref[0], 8)
        dfalse_h = jax.lax.broadcasted_iota(jnp.int32, (R // 2, 128), 1) < z_ref[0]
        seq = [[15], [14, 0], [13, 1], [12, 2], [11, 3], [10, 4], [9, 5], [8, 6], [7]]
        items = [(hh, rs) for hh in range(2) for rs in seq]
        n_items = len(items)

        def attention(p, extra=None):
            pins = {}

            def stage_a(t):
                hh, rs = items[t]
                sb = sbufs[t % NB]
                off = 0
                for pi, r in enumerate(rs):
                    W = R * (r + 1)
                    qu = q_s[hh, r * R // 2:(r + 1) * R // 2, :]
                    if (t - PIN) in pins and pi == 0:
                        for o_prev in pins[t - PIN]:
                            qu = jnp.where(dfalse_h, o_prev, qu)
                    qv = _upk(qu)
                    mx = None
                    for c0 in range(0, W, KC):
                        w = min(KC, W - c0)
                        sc_ = _dot_nt(qv, _upk(k_s[hh, c0 // 2:(c0 + w) // 2, :]))
                        for c1 in range(0, w, 128):
                            tile = sc_[:, c1:c1 + 128]
                            kk = c0 + c1
                            if kk == r * R:
                                tile = jnp.minimum(tile, cap_s[...])
                            sb[:, off + kk:off + kk + 128] = tile
                            mx = tile if mx is None else jnp.maximum(mx, tile)
                    mrow = jnp.max(mx, axis=-1, keepdims=True)
                    mbufs[t % NB][:, pi * 128:(pi + 1) * 128] = jnp.broadcast_to(mrow, (R, 128))
                    off += W

            def stage_f(t):
                hh, rs = items[t]
                sb = sbufs[t % NB]
                off = 0
                pins[t] = []
                for pi, r in enumerate(rs):
                    W = R * (r + 1)
                    mn = mbufs[t % NB][pl.ds(zld, R), pi * 128:(pi + 1) * 128]
                    psum = None
                    pv = None
                    for c0 in range(0, W, KC):
                        w = min(KC, W - c0)
                        prs = []
                        for c1 in range(0, w, 128):
                            kk = off + c0 + c1
                            pr = jnp.exp2(sb[pl.ds(zld, R), kk:kk + 128] - mn)
                            psum = pr if psum is None else psum + pr
                            prs.append(pr)
                        pm = (prs[0] if len(prs) == 1 else jnp.concatenate(prs, axis=1)).astype(BF16)
                        d = _dot(pm, _upk(v_s[hh, c0 // 2:(c0 + w) // 2, :]))
                        pv = d if pv is None else pv + d
                    lt = jnp.sum(psum, axis=-1, keepdims=True)
                    r0_ = pl.reciprocal(lt, approx=True)
                    rl = r0_ * (2.0 - lt * r0_)
                    o = _pk(pv * rl)
                    pins[t].append(o)
                    ctx_s[p, r * R // 2:(r + 1) * R // 2, hh * D:(hh + 1) * D] = o
                    off += W

            for t in range(n_items + 1):
                if t < n_items:
                    stage_a(t)
                if extra is not None and t in extra:
                    extra[t]()
                if t >= 1:
                    stage_f(t - 1)

        def pair_body(p, _):
            nslot = (p + 1) % 2
            for cp in raw_copies(p + 1, nslot):
                cp.wait()
            for cp in raw_copies(jnp.minimum(p + 2, NP - 1), p % 2):
                cp.start()

            def wait_unpack():
                unpack(nslot)
            pieces = []
            for i in range(S // PROJ_RB - 1, -1, -1):
                pieces.append(lambda i=i: proj_kv(i * PROJ_RB, PROJ_RB))
                pieces.append(lambda i=i: proj_q(i * PROJ_RB, PROJ_RB))
            extra = {3: wait_unpack, n_items - 1: pieces[0], n_items: pieces[1]}
            used = 2
            attention(p, extra)
            for f in pieces[used:]:
                f()
            return _

        for cp in late:
            cp.start()
        jax.lax.fori_loop(0, NP - 1, pair_body, None)
        for cp in raw_copies(NP - 1, (NP - 2) % 2):
            cp.wait()
        attention(NP - 1)

        for cp in late:
            cp.wait()
        mod2 = _dot(sc16, wm2_s[...])[0:8].astype(BF16).astype(F32)
        mod_s[...] = mod2

        g_s[0:8, :] = jnp.zeros((8, M), F32)
        g_s[8 + S:16 + S, :] = jnp.zeros((8, M), F32)

        HB1 = EP_RB // EPH1

        def ep1_body(r, _):
            halves = []
            for hf in range(EPH1):
                r0 = pl.multiple_of(r * EP_RB + hf * HB1, HB1)
                rs = pl.ds(r0, HB1)
                rs2 = pl.ds(pl.multiple_of(r * (EP_RB // 2) + hf * (HB1 // 2), HB1 // 2), HB1 // 2)
                cx = jnp.concatenate([_upk(ctx_s[pp, rs2, :]) for pp in range(NP)], axis=1)
                halves.append((r0, rs, x_s[rs, :], _dot(cx, wo_s[...])))
            ga = mod_s[0:1, 0:M]
            sb_ = mod_s[0:1, M:2 * M]
            cb = mod_s[0:1, 2 * M:3 * M]
            outs = []
            for (r0, rs, xin, acc) in halves:
                x1 = xin.astype(F32) + ga * acc
                hb = _ln(x1) * (1.0 + cb) + sb_
                pre = _dot(_ln(hb).astype(BF16), w1_s[...])
                outs.append((r0, rs, x1, hb, pre))
            for (r0, rs, x1, hb, pre) in outs:
                g = _gelu(pre)
                x1_s[rs, :] = x1
                hb_s[rs, :] = hb
                g_s[pl.ds(r0 + 8, HB1), :] = g
            return _

        HB2 = EP_RB // EPH

        def out_copy(b, slot, hf):
            return pltpu.make_async_copy(
                o_s.at[slot, pl.ds(hf * HB2, HB2), :],
                out_hbm.at[pl.ds(pl.multiple_of(b * EP_RB + hf * HB2, HB2), HB2), :], osems.at[slot, hf])


        def ep2_body(r, _):
            @pl.when(r >= 2)
            def _w():
                for hf in range(EPH):
                    out_copy(r - 2, r % 2, hf).wait()
            lane = jax.lax.broadcasted_iota(jnp.int32, (HB2, 128), 1)
            gb = mod_s[0:1, 3 * M:4 * M]
            st1 = []
            for hf in range(EPH):
                r0 = pl.multiple_of(r * EP_RB + hf * HB2, HB2)
                rs = pl.ds(r0, HB2)
                wins = {c0: g_s[pl.ds(r0, HB2 + 16), c0:c0 + 128] for c0 in range(0, M, 128)}
                gm1 = lambda c0: wins[c0][7:7 + HB2]
                gp1 = lambda c0: wins[c0][9:9 + HB2]
                gm2 = lambda c0: wins[c0][6:6 + HB2]
                gp2 = lambda c0: wins[c0][10:10 + HB2]
                t0 = gm1(0)
                t1 = jnp.where(lane < 32, gm1(128), gp1(128))
                t2 = jnp.where(lane < 64, gp1(256), gm2(256))
                t3 = jnp.where(lane < 96, gm2(384), gp2(384))
                t4 = gp2(512)
                gs = jnp.concatenate([t0, t1, t2, t3, t4], axis=1).astype(BF16)
                st1.append((rs, hb_s[rs, :], x1_s[rs, :], _dot(gs, w2_s[...])))
            st2 = []
            for (rs, hbv, x1v, hs) in st1:
                xb = hbv + hs
                u = _gelu(_dot_nt(_ln(xb).astype(BF16), w3_s[...])).astype(BF16)
                st2.append((xb, x1v, u))
            for hf, (xb, x1v, u) in enumerate(st2):
                h2 = _dot(u, w4_s[...])
                o_s[r % 2, hf * HB2:(hf + 1) * HB2, :] = (x1v + gb * (xb + h2)).astype(BF16)
                out_copy(r, r % 2, hf).start()
            return _

        NE = S // EP_RB
        jax.lax.fori_loop(0, NE, ep1_body, None)
        jax.lax.fori_loop(0, NE, ep2_body, None)
        for r in (NE - 2, NE - 1):
            for hf in range(EPH):
                out_copy(r, r % 2, hf).wait()

    return kernel


def run(A_x, A_c_kv, A_w_q, A_w_uk, A_w_uv, A_w_o, B_x, B_w1, B_w2, B_w3, B_w4, c, w_mod):
    del B_x
    hbm = pl.BlockSpec(memory_space=pltpu.HBM)
    out = pl.pallas_call(
        make_kernel(),
        out_shape=jax.ShapeDtypeStruct((S, M), BF16),
        in_specs=[hbm] * 10 + [pl.BlockSpec(memory_space=pltpu.VMEM), hbm, pl.BlockSpec(memory_space=pltpu.SMEM)],
        out_specs=hbm,
        scratch_shapes=[
            pltpu.VMEM((S, M), BF16), pltpu.VMEM((S, DC), BF16),
            pltpu.VMEM((H * D, M), BF16),
            pltpu.VMEM((M, M), BF16), pltpu.VMEM((M, M), BF16),
            pltpu.VMEM((F, M), BF16), pltpu.VMEM((F, M), BF16),
            pltpu.VMEM((M, 2 * M), BF16), pltpu.VMEM((M, 4 * M), BF16),
            pltpu.VMEM((2, M, D), U32), pltpu.VMEM((2, DC, D), U32), pltpu.VMEM((2, DC, D), U32),
            pltpu.VMEM((M // 2, 2 * D), U32), pltpu.VMEM((DC // 2, 4 * D), U32),
            pltpu.VMEM((8, 4 * M), F32),
            pltpu.VMEM((S // 2, M), U32),
            pltpu.VMEM((2, S // 2, D), U32), pltpu.VMEM((2, S // 2, D), U32), pltpu.VMEM((2, S // 2, D), U32),
            pltpu.VMEM((NP, S // 2, 2 * D), U32),
            pltpu.VMEM((S, M), F32),
            pltpu.VMEM((S, M), F32),
            pltpu.VMEM((S + 16, M), F32),
            pltpu.VMEM((2, EP_RB, M), BF16),
            pltpu.VMEM((R, 128), F32),
            pltpu.SemaphoreType.DMA((11,)),
            pltpu.SemaphoreType.DMA((2, 3)),
            pltpu.SemaphoreType.DMA((2, EPH)),
        ] + [pltpu.VMEM((R, S), F32)] * NB + [pltpu.VMEM((R, 256), F32)] * NB,
        compiler_params=pltpu.CompilerParams(
            vmem_limit_bytes=120 * 1024 * 1024,
            flags={"XLA_TPU_FORCE_LP_LLO_SCHEDULER": True},
            disable_bounds_checks=True),
    )(A_x.reshape(S, M), A_c_kv.reshape(S, DC), A_w_q, A_w_uk, A_w_uv, A_w_o.reshape(H * D, M),
      B_w1, B_w2, B_w3.T, B_w4, c, w_mod, np.zeros((1,), np.int32))
    return out.reshape(1, S, M)


@jax.jit
def pallas_adaLN_cond__compressed_kv_cla__mixer_s_mlp__prompt_kernel(
    A_x: jax.Array,
    A_c_kv: jax.Array,
    A_w_q: jax.Array,
    A_w_uk: jax.Array,
    A_w_uv: jax.Array,
    A_w_o: jax.Array,
    B_x: jax.Array,
    B_w1: jax.Array,
    B_w2: jax.Array,
    B_w3: jax.Array,
    B_w4: jax.Array,
    c: jax.Array,
    w_mod: jax.Array,
):
    return run(A_x, A_c_kv, A_w_q, A_w_uk, A_w_uv, A_w_o, B_x, B_w1, B_w2, B_w3, B_w4, c, w_mod)
```
